```python
import os as _os
_os.environ.setdefault("JAX_PLATFORMS", "cpu")
import jax
import jax.numpy as jnp

def _softmax(x, axis=-1):
    return jax.nn.softmax(x, axis=axis)
def _gelu(x):
    return jax.nn.gelu(x, approximate=True)
def _silu(x):
    return jax.nn.silu(x)
def _sigmoid(x):
    return jax.nn.sigmoid(x)
def _layernorm(x, axis=-1, eps=1e-5):
    m = jnp.mean(x, axis=axis, keepdims=True)
    v = jnp.var(x, axis=axis, keepdims=True)
    return (x - m) / jnp.sqrt(v + eps)
def _scatter_add(tgt, idx, src, axis=0):
    return tgt.at[idx].add(src)
def _segment_sum(src, seg, n):
    return jax.ops.segment_sum(src, seg, n)
class _Rng:
    def __init__(self, key):
        self._k = key
    def _next(self):
        self._k, sub = jax.random.split(self._k)
        return sub
    def normal(self, shape):
        return jax.random.normal(self._next(), shape, dtype=jnp.bfloat16)
    def randint(self, lo, hi, shape):
        return jax.random.randint(self._next(), shape, lo, hi, dtype=jnp.int32)
    def uniform(self, shape, lo=0.0, hi=1.0):
        return jax.random.uniform(self._next(), shape, jnp.bfloat16, lo, hi)
    def permutation(self, n):
        return jax.random.permutation(self._next(), n)


kernel_name = 'sequential_preLN__softmax_full_mha__dense_activation_gelu__prompt'

def setup_inputs():
    _rng = _Rng(jax.random.key(int.from_bytes(__import__("os").urandom(4), "little")))
    _w = (lambda a: (lambda t: t.astype(jnp.bfloat16) if jnp.issubdtype(t.dtype, jnp.floating) else t)(jnp.asarray(a)))
    def _A_setup():
        B, S, D = 1, 2048, 512
        return {
            "x": _w((lambda *s: _rng.normal(s) * 0.05)(B, S, D)),
            "wqkv": _w((lambda *s: _rng.normal(s) * 0.05)(D, 3 * D)),
            "wo": _w((lambda *s: _rng.normal(s) * 0.05)(D, D)),
        }
    _A_in = _A_setup()

    def _B_setup():
        B, S, D, F = 1, 2048, 512, 1792
        return {
            "x": _w((lambda *s: _rng.normal(s) * 0.05)(B, S, D)),
            "w1": _w((lambda *s: _rng.normal(s) * 0.4)(D, F) * (D ** -0.5)),
            "b1": _w((lambda *s: _rng.normal(s) * 0.4)(F) * 0.01),
            "w2": _w((lambda *s: _rng.normal(s) * 0.4)(F, D) * (F ** -0.5)),
            "b2": _w((lambda *s: _rng.normal(s) * 0.05)(D) * 0.01),
        }
    _B_in = _B_setup()

    return {
        "A_x": _A_in["x"],
        "A_wqkv": _A_in["wqkv"],
        "A_wo": _A_in["wo"],
        "B_x": _B_in["x"],
        "B_w1": _B_in["w1"],
        "B_b1": _B_in["b1"],
        "B_w2": _B_in["w2"],
        "B_b2": _B_in["b2"],
    }

def reference(A_x, A_wqkv, A_wo, B_x, B_w1, B_b1, B_w2, B_b2):
    def _A_ref(x, wqkv, wo):
        B, S, D = x.shape
        H = 32; Dh = D // H
        qkv = (lambda x, *d: x.transpose(*d))((x @ wqkv).reshape(B, S, 3, H, Dh), 2, 0, 3, 1, 4)
        q, k, v = qkv[0], qkv[1], qkv[2]
        scale = Dh ** -0.5
        scores = jnp.einsum("bhqd,bhkd->bhqk", q, k) * scale
        p = _softmax(scores, axis=-1)
        o = jnp.einsum("bhqk,bhkd->bhqd", p, v)
        return (lambda x, *d: x.transpose(*d))(o, 0, 2, 1, 3).reshape(B, S, D) @ wo

    def _B_ref(x, w1, b1, w2, b2):
        h = jnp.einsum("bsd,df->bsf", x, w1) + b1
        h = _gelu(h)
        return jnp.einsum("bsf,fd->bsd", h, w2) + b2

    x = A_x
    h = x + _A_ref(_layernorm(x, axis=-1), A_wqkv, A_wo)
    h2 = h + _B_ref(_layernorm(h, axis=-1), B_w1, B_b1, B_w2, B_b2)
    return h2
```

```python
import functools
import math
import jax
import jax.numpy as jnp
from jax import lax
import jax.experimental.pallas as pl
import jax.experimental.pallas.tpu as pltpu

H = 32
EPS = 1e-5
LANES = 128
BQ = 512
KC = 128
VK = 16
SHIFT = 32
PF32 = 0
PIECE = "quad"
RC = 512
SAFE_LOG2 = 64.0
f32 = jnp.float32
bf16 = jnp.bfloat16
u32 = jnp.uint32


def _layernorm(x):
    m = jnp.mean(x, axis=-1, keepdims=True)
    xc = x - m
    v = jnp.mean(xc * xc, axis=-1, keepdims=True)
    return xc * lax.rsqrt(v + EPS)


def _gelu(u):
    c0 = math.sqrt(2.0 / math.pi)
    c1 = c0 * 0.044715
    t = jnp.tanh(u * (c0 + c1 * (u * u)))
    hu = 0.5 * u
    return hu + hu * t


def _rows8(x):
    return [x[i * 8:(i + 1) * 8] for i in range(x.shape[0] // 8)]


def _pack(x):
    return pltpu.bitcast(x.astype(bf16), u32)


def _unpack(w):
    return pltpu.bitcast(w, bf16)


def _dot(a, b):
    return jnp.dot(a, b, preferred_element_type=f32)


def _dot_nt(a, b):
    return lax.dot_general(a, b, (((1,), (1,)), ((), ())), preferred_element_type=f32)


def _kernel(x_hbm, wqkv_hbm, wo_hbm, w1_hbm, b1_ref, w2_hbm, b2_ref, out_hbm,
            x_v, wqkv_v, wo_v, w1_v, w2_v, wqt_s, wvt_s, k_s, qt_s, vt_s, ot_s,
            kh_a, kh_b, kb_a, kb_b, qb_a, qb_b, s_s, out_v, in_sem, out_sem):
    S, D = x_v.shape
    Dh = D // H
    n_rc = S // RC
    n_qb = S // BQ
    n_kt = S // KC
    n_qt = BQ // LANES
    hpg = LANES // Dh
    MK = KC - VK
    qscale = (Dh ** -0.5) * math.log2(math.e)

    x_cp = [pltpu.make_async_copy(x_hbm.at[pl.ds(r * RC, RC)], x_v.at[pl.ds(r * RC, RC)], in_sem.at[r])
            for r in range(n_rc)]
    w_cp = [pltpu.make_async_copy(src, dst, in_sem.at[n_rc + i])
            for i, (src, dst) in enumerate([(wqkv_hbm, wqkv_v), (wo_hbm, wo_v), (w1_hbm, w1_v), (w2_hbm, w2_v)])]
    x_cp[0].start()
    w_cp[0].start()
    for c in x_cp[1:] + w_cp[1:]:
        c.start()

    def prep_head(h, kh_ref, kb_ref):
        kh = pltpu.roll(k_s[h // hpg], (LANES - (h % hpg) * Dh) % LANES, 1)
        kh_ref[...] = kh
        if VK:
            for j in range(n_kt):
                kv = _unpack(kh[(j * KC + MK) // 2:(j + 1) * KC // 2]).astype(f32)
                for d in range(Dh):
                    kb_ref[0, d, j * VK:(j + 1) * VK, :] = jnp.broadcast_to(kv[:, d:d + 1], (VK, LANES))

    def q_rows(h, qb):
        return qt_s[qb, pl.ds(pl.multiple_of(h * (Dh // 2), Dh // 2), Dh // 2), :]

    def prep_item(h, qb, qb_ref):
        if VK:
            qh = _unpack(q_rows(h, qb)).astype(f32)
            for d in range(Dh):
                qb_ref[0, d] = jnp.broadcast_to(qh[d:d + 1], (8, BQ))

    w_cp[0].wait()
    wqt_s[...] = pltpu.bitcast(wqkv_v[:, 0:D].T, u32)
    wvt_s[...] = pltpu.bitcast(wqkv_v[:, 2 * D:3 * D].T, u32)
    kn = qn = vn = None
    for r in range(n_rc):
        x_cp[r].wait()
        rows = pl.ds(r * RC, RC)
        xn = _layernorm(x_v[rows, :].astype(f32)).astype(bf16)
        k = _dot(xn, wqkv_v[:, D:2 * D])
        kp = _pack(k)
        for g in range(D // LANES):
            k_s[g, pl.ds(r * RC // 2, RC // 2), :] = kp[:, g * LANES:(g + 1) * LANES]
        qt = _dot_nt(_unpack(wqt_s[...]), xn) * qscale
        qt_s[r] = _pack(qt)
        vt = _dot_nt(_unpack(wvt_s[...]), xn)
        vt_s[:, rows] = vt if PF32 else _pack(vt)
        k2 = _rows8(k * k)
        for i in range(0, len(k2), 16):
            w = functools.reduce(jnp.maximum, k2[i:i + 16])
            for g in range(D // LANES):
                wg = w[:, g * LANES:(g + 1) * LANES]
                for sh in (1, 2, 4, 8):
                    wg = wg + pltpu.roll(wg, sh, 1)
                kn = wg if kn is None else jnp.maximum(kn, wg)
        q2 = _rows8(qt * qt)
        for i in range(0, len(q2), 2):
            w = q2[i] + q2[i + 1]
            w = functools.reduce(jnp.maximum, [w[:, j * LANES:(j + 1) * LANES] for j in range(RC // LANES)])
            w = jnp.sum(w, axis=0, keepdims=True)
            qn = w if qn is None else jnp.maximum(qn, w)
        w = functools.reduce(jnp.maximum, _rows8(jnp.abs(vt)))
        vn = w if vn is None else jnp.maximum(vn, w)
    prep_head(0, kh_a, kb_a)
    prep_item(0, 0, qb_a)
    safe = jnp.logical_and(jnp.max(kn) * jnp.max(qn) <= SAFE_LOG2 * SAFE_LOG2, jnp.max(vn) <= 2.0 ** 40)

    def v_rows(h, j):
        n = Dh if PF32 else Dh // 2
        return vt_s[pl.ds(pl.multiple_of(h * n, n), n), pl.ds(j * KC, KC)]

    def finish(h, qb, l, acc):
        o = acc * (1.0 / jnp.sum(l, axis=0, keepdims=True))
        ot_s[qb, pl.ds(pl.multiple_of(h * (Dh // 2), Dh // 2), Dh // 2), :] = _pack(o)

    def fast_pair(i, _):
        n_it = 2 * n_qb
        T = n_it * n_kt
        heads = [2 * i, 2 * i + 1]
        khs, kbs, qbs = [kh_a, kh_b], [kb_a, kb_b], [qb_a, qb_b]
        keep = lax.broadcasted_iota(jnp.int32, (8, LANES), 0) > (i // 65536 - 1)

        def zero(t):
            return (i * 1024 + t) // 65536

        blocks = [j * KC + b * 16 for j in range(n_kt) for b in reversed(range(MK // 16))]
        ends = [min((j + 1) * (MK // 16) + SHIFT // 16, len(blocks)) for j in range(n_kt - 1)] + [len(blocks)]
        starts = [0] + ends[:-1]
        if PIECE == "quad":
            shape = [[(r, q, range(a * 4, a * 4 + 4)) for r in range(2) for q in (qq, qq + 1)]
                     for qq in (0, 2) for a in range(4)]
        else:
            shape = [[(r, q, range(a * 8, a * 8 + 8)) for r in range(2)] for q in range(n_qt) for a in range(2)]
        pieces = [(u, j, pc) for u in range(n_it) for j in range(n_kt) for pc in shape] if VK else []
        anchors, tm = [], 0
        for t in range(T):
            j = t % n_kt
            for b in range(starts[j], ends[j]):
                anchors.append((("k", t, b), tm))
                tm += 16
            if t >= 1:
                anchors.append((("v", t - 1), tm))
                tm += 16
        assign = {}
        for n, pc in enumerate(pieces):
            target = (n + 0.5) * tm / len(pieces)
            best = min(anchors, key=lambda a: abs(a[1] - target))
            assign.setdefault(best[0], []).append(pc)
        partial = {}

        def run_piece(u, j, pc):
            kb_ref, qb_ref = kbs[u // n_qb], qbs[u % 2]
            z = zero(u * n_kt + j)
            accs = partial.setdefault((u, j), {})
            for d in pc[0][2]:
                for (r, q, _) in pc:
                    term = kb_ref[z, d, pl.ds(j * VK + r * 8, 8), :] * qb_ref[z, d, :, pl.ds(q * LANES, LANES)]
                    accs[r, q] = term if d == 0 else accs[r, q] + term
            return accs[pc[-1][0], pc[-1][1]]

        def anchored(x, key):
            dep = None
            for pc in assign.pop(key, []):
                dep = run_piece(*pc)
            if dep is None:
                return x
            return jnp.where(keep, x, dep if x.dtype == f32 else pltpu.bitcast(dep, u32))

        lane = lax.broadcasted_iota(jnp.int32, (8, LANES), 1)

        def prep_piece(u, j, dep):
            nh = u // n_qb + 1
            hn = jnp.minimum(2 * i + nh, H - 1)
            g, lo = hn // hpg, (hn % hpg) * Dh
            n = (u % n_qb) * n_kt + j
            idx = jnp.where(keep, (lane + lo) % LANES, dep)
            for r in range(2 * n, 2 * n + 2):
                khs[nh % 2][pl.ds(r * 8, 8), :] = jnp.take_along_axis(k_s[g, pl.ds(r * 8, 8), :], idx, axis=1)
            if VK:
                d = n // 4
                idx = jnp.where(keep, jnp.full((8, LANES), lo + d, jnp.int32), dep)
                for jj in range(4 * (n % 4), 4 * (n % 4) + 4):
                    w = jnp.take_along_axis(k_s[g, pl.ds((jj * KC + MK) // 2, 8), :], idx, axis=1)
                    kbs[nh % 2][0, d, pl.ds(jj * VK, VK), :] = _unpack(w).astype(f32)
                un = u + 1
                qw = q_rows(jnp.minimum(2 * i + un // n_qb, H - 1), un % n_qb + zero(u * n_kt + j))
                for q in range(n_qt):
                    w = jnp.where(keep, qw[:, q * LANES:(q + 1) * LANES], pltpu.bitcast(dep, u32))
                    row = _unpack(w).astype(f32)[j:j + 1]
                    qbs[un % 2][0, j, :, pl.ds(q * LANES, LANES)] = jnp.broadcast_to(row, (8, LANES))

        sv = {}
        l = acc = None
        for t in range(T + 1):
            if t < T:
                u, j = divmod(t, n_kt)
                h, qb = heads[u // n_qb], u % n_qb
                lhs = [anchored(khs[u // n_qb][pl.ds(blocks[b] // 2, 8), :], ("k", t, b))
                       for b in range(starts[j], ends[j])]
                s = _dot(_unpack(jnp.concatenate(lhs, axis=0))[:, :Dh], _unpack(q_rows(h, qb + zero(t))))
                for n, b in enumerate(range(starts[j], ends[j])):
                    sv[u, blocks[b]] = s[n * 16:(n + 1) * 16]
                prep_piece(u, j, pltpu.bitcast(s[0:8, 0:LANES], jnp.int32))
            if t >= 1:
                u, j = divmod(t - 1, n_kt)
                h, qb = heads[u // n_qb], u % n_qb
                vt = v_rows(h, j)
                if PF32:
                    vt = jnp.concatenate([anchored(vt[0:8], ("v", t - 1)), vt[8:16]], axis=0)
                else:
                    vt = anchored(vt, ("v", t - 1))
                rows = [sv.pop((u, j * KC + b * 16)) for b in range(MK // 16)]
                if VK:
                    a = partial.pop((u, j))
                    rows += [jnp.concatenate([a[r, q] for q in range(n_qt)], axis=1) for r in range(VK // 8)]
                p = jnp.exp2(jnp.concatenate(rows, axis=0))
                l = functools.reduce(jnp.add, ([] if j == 0 else [l]) + _rows8(p)[::-1])
                pv = _dot(vt, p) if PF32 else _dot(_unpack(vt), p.astype(bf16))
                acc = pv if j == 0 else acc + pv
                if j == n_kt - 1:
                    finish(h, qb, l, acc)
        assert not assign or not any(assign.values())

    def guarded_item(it, _):
        h, qb = it // n_qb, it % n_qb

        @pl.when(qb == 0)
        def _():
            kh_a[...] = pltpu.roll(k_s[h // hpg], (LANES - (h % hpg) * Dh) % LANES, 1)

        qh = _unpack(q_rows(h, qb))
        step = 4 * KC

        def scores(c, m):
            r0 = pl.multiple_of(c * step, step)
            s = _dot(_unpack(kh_a[pl.ds(pl.multiple_of(r0 // 2, step // 2), step // 2), :])[:, :Dh], qh)
            s_s[pl.ds(r0, step), :] = s
            return functools.reduce(jnp.maximum, [m] + _rows8(s))

        m = lax.fori_loop(0, S // step, scores, jnp.full((8, BQ), -jnp.inf, f32))
        m = jnp.max(m, axis=0, keepdims=True)

        def values(c, carry):
            l, acc = carry
            r0 = pl.multiple_of(c * step, step)
            p = jnp.exp2(s_s[pl.ds(r0, step), :] - m)
            n = Dh if PF32 else Dh // 2
            vt = vt_s[pl.ds(pl.multiple_of(h * n, n), n), pl.ds(r0, step)]
            pv = _dot(vt, p) if PF32 else _dot(_unpack(vt), p.astype(bf16))
            return functools.reduce(jnp.add, [l] + _rows8(p)), acc + pv

        l, acc = lax.fori_loop(0, S // step, values, (jnp.zeros((8, BQ), f32), jnp.zeros((Dh, BQ), f32)))
        finish(h, qb, l, acc)

    @pl.when(safe)
    def _():
        lax.fori_loop(0, H // 2, fast_pair, None)

    @pl.when(jnp.logical_not(safe))
    def _():
        lax.fori_loop(0, H * n_qb, guarded_item, None)

    for c in w_cp[1:]:
        c.wait()
    b1 = b1_ref[...].astype(f32)
    b2 = b2_ref[...].astype(f32)
    out_cp = [pltpu.make_async_copy(out_v.at[pl.ds(r * RC, RC)], out_hbm.at[pl.ds(r * RC, RC)], out_sem.at[r])
              for r in range(n_rc)]
    for r in range(n_rc):
        rows = pl.ds(r * RC, RC)
        o = _unpack(ot_s[r]).T
        hres = x_v[rows, :].astype(f32) + _dot(o, wo_v[...])
        hn = _layernorm(hres).astype(bf16)
        u = _dot(hn, w1_v[...]) + b1
        y = _dot(_gelu(u).astype(bf16), w2_v[...]) + b2
        out_v[rows, :] = (hres + y).astype(out_v.dtype)
        out_cp[r].start()
    for c in out_cp:
        c.wait()


@jax.jit
def pallas_sequential_preLN__softmax_full_mha__dense_activation_gelu__prompt_kernel(A_x, A_wqkv, A_wo, B_x, B_w1, B_b1, B_w2, B_b2):
    del B_x
    B, S, D = A_x.shape
    F = B_w1.shape[1]
    Dh = D // H
    n_rc = S // RC
    hbm = pl.BlockSpec(memory_space=pl.ANY)
    vmem = pl.BlockSpec(memory_space=pltpu.VMEM)
    V = pltpu.VMEM
    out = pl.pallas_call(
        _kernel,
        out_shape=jax.ShapeDtypeStruct((S, D), A_x.dtype),
        in_specs=[hbm, hbm, hbm, hbm, vmem, hbm, vmem],
        out_specs=hbm,
        scratch_shapes=[
            V((S, D), A_x.dtype), V((D, 3 * D), bf16), V((D, D), bf16), V((D, F), bf16), V((F, D), bf16),
            V((D // 2, D), u32), V((D // 2, D), u32),
            V((D // LANES, S // 2, LANES), u32),
            V((S // BQ, D // 2, BQ), u32),
            V((D, S), f32) if PF32 else V((D // 2, S), u32),
            V((S // BQ, D // 2, BQ), u32),
            V((S // 2, LANES), u32), V((S // 2, LANES), u32),
            V((1, Dh, max(S // KC * VK, 8), LANES), f32), V((1, Dh, max(S // KC * VK, 8), LANES), f32),
            V((1, Dh, 8, BQ), f32), V((1, Dh, 8, BQ), f32),
            V((S, BQ), f32),
            V((S, D), A_x.dtype),
            pltpu.SemaphoreType.DMA((n_rc + 4,)),
            pltpu.SemaphoreType.DMA((n_rc,)),
        ],
        compiler_params=pltpu.CompilerParams(vmem_limit_bytes=100 * 1024 * 1024),
        name="fused_block",
    )(A_x.reshape(S, D), A_wqkv, A_wo, B_w1, B_b1.reshape(1, F), B_w2, B_b2.reshape(1, D))
    return out.reshape(B, S, D)
```

```python
import functools
import math
import jax
import jax.numpy as jnp
from jax import lax
import jax.experimental.pallas as pl
import jax.experimental.pallas.tpu as pltpu

H = 32
EPS = 1e-5
LANES = 128
BQ = 512
KC = 128
VP = [int(v) for v in "16".split(",")]
LAGB = 9
PF32 = 0
PIECE = "pair"
NANC = 2
LEAD = 32
ONLY = ""
NH = 2
FRONT = 0
BACK = 1
STR = 1
OPH = 1
OPG = 3
RL0 = 0
RL1 = 6
ORD1 = [int(c) for c in "2413065"]
ORD2 = [int(c) for c in "2504163"]
KPS = 52
QPS = 12
QP0 = 1
KP0 = 1
PVD = 10
PVALL = 1
RC = 512
SAFE_LOG2 = 64.0
f32 = jnp.float32
bf16 = jnp.bfloat16
u32 = jnp.uint32
i32 = jnp.int32


def _layernorm(x):
    m = jnp.mean(x, axis=-1, keepdims=True)
    xc = x - m
    v = jnp.mean(xc * xc, axis=-1, keepdims=True)
    return xc * lax.rsqrt(v + EPS)


def _gelu2(u):
    c0 = math.sqrt(2.0 / math.pi)
    c1 = c0 * 0.044715
    return u + u * jnp.tanh(u * (c0 + c1 * (u * u)))


def _gelu(u):
    c0 = math.sqrt(2.0 / math.pi)
    c1 = c0 * 0.044715
    t = jnp.tanh(u * (c0 + c1 * (u * u)))
    hu = 0.5 * u
    return hu + hu * t


def _rows8(x):
    return [x[i * 8:(i + 1) * 8] for i in range(x.shape[0] // 8)]


def _pack(x):
    return pltpu.bitcast(x.astype(bf16), u32)


def _unpack(w):
    return pltpu.bitcast(w, bf16)


def _dot(a, b):
    return jnp.dot(a, b, preferred_element_type=f32)


def _dot_nt(a, b):
    return lax.dot_general(a, b, (((1,), (1,)), ((), ())), preferred_element_type=f32)


def _lane_gather(x, idx):
    return jnp.take_along_axis(x, idx, axis=1, mode="promise_in_bounds")


def _kernel(x_hbm, wqkv_hbm, wo_hbm, w1_hbm, b1_hbm, w2_hbm, b2_hbm, out_hbm, *scratch):
    if FRONT:
        b1_ref, *scratch = scratch
    else:
        *scratch, b1_ref = scratch
    *scratch, b2_ref = scratch
    _body(x_hbm, wqkv_hbm, wo_hbm, w1_hbm, b1_hbm, w2_hbm, b2_hbm, out_hbm, b1_ref, b2_ref, *scratch)


def _body(x_hbm, wqkv_hbm, wo_hbm, w1_hbm, b1_hbm, w2_hbm, b2_hbm, out_hbm, b1_ref, b2_ref,
            x_v, wqkv_v, wo_v, w1_v, w2_v, wqt_s, wvt_s, xn_0, xn_1, xn_2, xn_3, k_s, kv_s, qt_s, qf_s, vt_s, ot_s, l_s,
            kh_a, kh_b, kb_a, kb_b, qb_a, qb_b, pend_s, s_s, w1t_s, w2t_s, h_s, o_0, o_1, o_2, o_3, a1_0, a1_1, a1_2, a1_3, a2_s, out_v, zero_s, in_sem, out_sem):
    S, D = x_v.shape
    xn_s = [xn_0, xn_1, xn_2, xn_3]
    o_s = [o_0, o_1, o_2, o_3]
    a1_s = [a1_0, a1_1, a1_2, a1_3]
    Dh = D // H
    n_rc = S // RC
    n_qb = S // BQ
    n_kt = S // KC
    n_qt = BQ // LANES
    hpg = LANES // Dh
    vk = [VP[j % len(VP)] for j in range(n_kt)]
    voff = [sum(vk[:j]) for j in range(n_kt + 1)]
    qscale = (Dh ** -0.5) * math.log2(math.e)

    def copy(src, dst, n):
        return pltpu.make_async_copy(src, dst, in_sem.at[n])

    def wqkv_cols(n):
        return copy(wqkv_hbm.at[:, pl.ds(n * D, D)], wqkv_v.at[n], n)

    x_cp = [copy(x_hbm.at[pl.ds(r * RC, RC)], x_v.at[pl.ds(r * RC, RC)], 8 + r) for r in range(n_rc)]
    wq_cp, wk_cp, wv_cp = wqkv_cols(0), wqkv_cols(1), wqkv_cols(2)
    ffn_cp = [copy(wo_hbm, wo_v, 3), copy(w1_hbm, w1_v, 4), copy(w2_hbm, w2_v, 5), copy(b1_hbm, b1_ref.at[pl.ds(0, b1_hbm.shape[0])], 6), copy(b2_hbm, b2_ref.at[pl.ds(0, D)], 7)]

    for c in [x_cp[0], wk_cp] + x_cp[1:] + [wq_cp, wv_cp] + ffn_cp:
        c.start()

    def put_zero(n, _):
        zero_s[n] = n // 65536

    lax.fori_loop(0, zero_s.shape[0], put_zero, None)
    zero0 = zero_s[0]
    keep0 = lax.broadcasted_iota(i32, (8, LANES), 0) >= zero0

    def q_rows(h, qb):
        return qt_s[qb, pl.ds(pl.multiple_of(h * (Dh // 2), Dh // 2), Dh // 2), :]

    P0 = ONLY in ("", "p0")
    def held(x, dep):
        if dep is None:
            return x
        head = jnp.concatenate([jnp.where(keep0, t, dep) for t in _rows8(x[:, :LANES])], axis=0)
        return jnp.concatenate([head, x[:, LANES:]], axis=1) if x.shape[1] > LANES else head

    def dot_after(dot, lhs_words, rhs, jobs):
        if not jobs:
            return dot(_unpack(lhs_words), rhs)
        rows = []
        for b in range(lhs_words.shape[0] // 8):
            cols = []
            for k in range(lhs_words.shape[1] // LANES):
                w = lhs_words[b * 8:(b + 1) * 8, k * LANES:(k + 1) * LANES]
                if (b, k) in jobs:
                    w = jnp.where(keep0, w, jobs[b, k]())
                cols.append(w)
            rows.append(jnp.concatenate(cols, axis=1))
        return dot(_unpack(jnp.concatenate(rows, axis=0)), rhs)

    norms = {}

    def bound(name, w):
        norms[name] = w if name not in norms else jnp.maximum(norms[name], w)

    def norm_rows(r0, n, dep=None):
        xn = _layernorm(held(x_v[pl.ds(r0, n), :].astype(f32), dep))
        xn_s[r0 // RC][0, pl.ds(r0 % RC // 2, n // 2), :] = _pack(xn)

    k_peaks = []

    def project_k(r, g, ln_rows=()):
        kg = _dot(_unpack(xn_s[r][g * zero0]), wqkv_v[1, :, pl.ds(g * LANES, LANES)])
        for n, (r0, wait) in enumerate(ln_rows):
            t = n * (RC // 8) // len(ln_rows) * 8
            norm_rows(r0, 32, kg[t:t + 8] if wait else None)
        k_s[g, pl.ds(r * RC // 2, RC // 2), :] = _pack(kg)
        for jj in range(RC // KC):
            j = r * RC // KC + jj
            kv_s[g, pl.ds(voff[j], vk[j]), :] = kg[jj * KC:jj * KC + vk[j]]
        k2 = _rows8(kg * kg)
        k_peaks.extend(functools.reduce(jnp.maximum, k2[n:n + 16]) for n in range(0, len(k2), 16))

    def project_q(r):
        qt = _dot_nt(_unpack(wqt_s[...]), _unpack(xn_s[r][0])) * qscale
        qt_s[r] = _pack(qt)
        qf_s[r] = qt
        q2 = _rows8(qt * qt)
        for n in range(0, len(q2), 2):
            w = q2[n] + q2[n + 1]
            w = functools.reduce(jnp.maximum, [w[:, j * LANES:(j + 1) * LANES] for j in range(RC // LANES)])
            bound("q", jnp.sum(w, axis=0, keepdims=True))

    def weight_combos(w_ref, t_ref, t, c, dep):
        kh, nh = w_ref.shape[0] // 2, w_ref.shape[1] // 2
        words = [pltpu.bitcast(w_ref[pl.ds(a * kh + t, 16), pl.ds(b * nh + c, LANES)], u32)
                 for a in range(2) for b in range(2)]
        dep = pltpu.bitcast(dep, u32)
        words = [jnp.where(keep0, w, dep) for w in words]
        b11, b12, b21, b22 = (_unpack(w).astype(f32) for w in words)
        for n, w in enumerate((_pack(b11 + b22), words[0], _pack(b12 - b22), _pack(b21 - b11),
                               words[3], _pack(b11 + b12), _pack(b21 + b22))):
            t_ref[n, pl.ds(t // 2, 8), pl.ds(c, LANES)] = w

    combo_jobs = [functools.partial(weight_combos, w_ref, t_ref, t, c)
                  for w_ref, t_ref in ((w1_v, w1t_s), (w2_v, w2t_s))
                  for t in range(0, w_ref.shape[0] // 2, 16) for c in range(0, w_ref.shape[1] // 2, LANES)]

    def release(todo, y):
        tiles = [y[t:t + 8, c:c + LANES] for c in range(0, y.shape[1], LANES) for t in range(0, y.shape[0], 8)]
        for n, fn in enumerate(todo):
            fn(tiles[n * len(tiles) // len(todo)])

    def share(todo, n, parts):
        return todo[n * len(todo) // parts:(n + 1) * len(todo) // parts]

    def project_v(r):
        vt = _dot_nt(_unpack(wvt_s[...]), _unpack(xn_s[r][0]))
        release(share(combo_jobs, r, n_rc), vt)
        vt_s[:, pl.ds(r * RC, RC)] = vt if PF32 else _pack(vt)
        bound("v", functools.reduce(jnp.maximum, _rows8(jnp.abs(vt))))

    n_g = D // LANES
    def spread(r, parts, free=0):
        rows = [(r0, n >= free) for n, r0 in enumerate(range(r * RC, (r + 1) * RC, 32))]
        return [rows[n * len(rows) // parts:(n + 1) * len(rows) // parts] for n in range(parts)]

    x_cp[0].wait()
    if P0:
        norm_rows(0, RC)
    wk_cp.wait()
    if P0:
        project_k(0, 0)
        project_k(0, 1)
    x_cp[1].wait()
    x_cp[2].wait()
    if P0:
        ln = spread(1, 2, 3) + spread(2, 4)
        for n, (r, g) in enumerate([(0, 2), (0, 3), (1, 0), (1, 1), (1, 2), (1, 3)]):
            project_k(r, g, ln[n])
        project_k(2, 0)
    for c in (x_cp[3], wq_cp, wv_cp):
        c.wait()
    if P0:
        ln = spread(3, 3, 3)
        for g in range(1, n_g):
            project_k(2, g, ln[g - 1])
        for g in range(n_g):
            project_k(3, g)
        wqt_s[...] = pltpu.bitcast(wqkv_v[0].T, u32)
        wvt_s[...] = pltpu.bitcast(wqkv_v[2].T, u32)
        for w in k_peaks:
            for sh in (1, 2, 4, 8):
                w = w + pltpu.roll(w, sh, 1)
            bound("k", w)
        for r in range(n_rc):
            project_q(r)
        kh_a[...] = k_s[0]
        kv0 = kv_s[0]
        for d in range(Dh):
            kb_a[0, d] = jnp.broadcast_to(kv0[:, d:d + 1], kv0.shape)
            qb_a[0, d] = jnp.broadcast_to(qf_s[0, d:d + 1, :], (8, BQ))
    for c in ffn_cp:
        c.wait()
    if P0:
        for r in range(n_rc):
            project_v(r)
        safe = jnp.logical_and(jnp.max(norms["k"]) * jnp.max(norms["q"]) <= SAFE_LOG2 * SAFE_LOG2,
                               jnp.max(norms["v"]) <= 2.0 ** 40)
    else:
        safe = jnp.max(b1_ref[pl.ds(0, D)].astype(f32).reshape(1, -1)) < 100.0

    def v_rows(h, start, size):
        n = Dh if PF32 else Dh // 2
        return vt_s[pl.ds(pl.multiple_of(h * n, n), n), pl.ds(start, size)]

    def finish(h, qb, l, acc):
        ot_s[qb, pl.ds(pl.multiple_of(h * Dh, Dh), Dh), :] = acc
        l_s[qb, h] = l

    n_it = NH * n_qb
    khs, kbs, qbs = [kh_a, kh_b], [kb_a, kb_b], [qb_a, qb_b]
    blocks = [(u, j, j * KC + b) for u in range(-1, n_it + 1) for j in range(n_kt)
              for b in range(KC - 16, vk[j] - 1, -16)]
    tile_end = {}
    for n, (u, j, _) in enumerate(blocks):
        tile_end[u, j] = n + 1
    tiles = [(-1, n_kt - 1)] + [(u, j) for u in range(n_it) for j in range(n_kt)]
    first = tile_end[-1, n_kt - 2] + LAGB
    stream, n = [], first
    for tile in tiles[:-1]:
        stream += [("k", blocks[m]) for m in range(n, tile_end[tile] + LAGB)] + [("v", tile)]
        n = tile_end[tile] + LAGB
    pending_in = blocks[tile_end[-1, n_kt - 2]:first]
    pending_out = blocks[tile_end[n_it - 1, n_kt - 2]:n]

    def tile_pieces(j):
        if PIECE == "quad":
            return [(r, 16, qq, 2, range(a * 4, a * 4 + 4)) for r in range(0, vk[j], 16) for qq in (0, 2) for a in range(4)]
        if PIECE == "half":
            return [(r, 16, q, 1, range(a * 4, a * 4 + 4)) for r in range(0, vk[j], 16) for q in range(n_qt) for a in range(4)]
        return [(r, 16, q, 1, range(a * 8, a * 8 + 8)) for r in range(0, vk[j], 16) for q in range(n_qt) for a in range(2)]

    def run_piece(partial, u, j, pc, z):
        r0, nr, q0, nq, dims = pc
        kb_ref, qb_ref = kbs[(u // n_qb) % 2], qbs[u % 2]
        accs = partial.setdefault((u, j), {})
        for d in dims:
            kk = kb_ref[z, d, pl.ds(voff[j] + r0, nr), :]
            qq = qb_ref[z, d, :, pl.ds(q0 * LANES, nq * LANES)]
            if nq > 1:
                kk = jnp.concatenate([kk] * nq, axis=1)
            term = kk * jnp.concatenate([qq] * (nr // 8), axis=0)
            accs[r0, q0] = term if d == 0 else accs[r0, q0] + term
        a = accs[r0, q0]
        return [a[r:r + 8, c:c + LANES] for r in range(0, nr, 8) for c in range(0, nq * LANES, LANES)]

    def pv_tile(probs, partial, u, j, vt, l, acc):
        a = partial.pop((u, j))
        rows = [jnp.exp2(jnp.concatenate([a[r, q] for q in sorted(q for (rr, q) in a if rr == r)], axis=1))
                for r in range(0, vk[j], 16)]
        rows += [probs.pop((u, j, j * KC + b)) for b in range(vk[j], KC, 16)]
        p = jnp.concatenate(rows, axis=0)
        l = functools.reduce(jnp.add, ([] if j == 0 else [l]) + _rows8(p)[::-1])
        pv = _dot(vt, p) if PF32 else _dot(_unpack(vt), p.astype(bf16))
        return l, (pv if j == 0 else acc + pv)

    def fast_heads(i, carry):
        l, acc = carry
        row = lax.broadcasted_iota(i32, (8, LANES), 0)
        lane = lax.broadcasted_iota(i32, (8, LANES), 1)
        keep = [row > (i // 65536 - 1 - a) for a in range(NANC + 1)]

        def zero(t):
            return (i * 1024 + t) // 65536

        def head(u):
            return jnp.clip(NH * i + u // n_qb, 0, H - 1)

        pieces = [(u, j, pc) for (u, j) in tiles[:-1] for pc in tile_pieces(j)]
        assign = {}
        for n, pc in enumerate(pieces):
            slot = int((n + 1) * len(stream) / len(pieces) - 1 - LEAD / 16 + 0.5)
            slot = max(0, min(slot, stream.index(("v", pc[:2]))))
            assign.setdefault(slot, []).append(pc)
        partial, after = {}, {}

        def anchored(x, slot):
            deps = []
            for (u, j, pc) in assign.pop(slot, []):
                deps = run_piece(partial, u, j, pc, zero((u + 1) * n_kt + j))
            deps = deps[-NANC:] + after.pop(slot, [])
            for a, dep in enumerate(deps):
                x = jnp.where(keep[a], x, dep if x.dtype == f32 else pltpu.bitcast(dep, u32))
            return x

        def prep_piece(u, j, dep):
            nh = u // n_qb + 1
            hn = head(nh * n_qb)
            g, lo = hn // hpg, (hn % hpg) * Dh
            step = (u % n_qb) * n_kt + j
            mine = [b // 16 for (uu, _, b) in blocks if uu == 0]
            rs = [r for n, r in enumerate(mine) if KP0 + n * KPS // len(mine) == step]
            if rs:
                idx = jnp.where(keep[0], (lane + lo) & (LANES - 1), pltpu.bitcast(dep, i32))
                for r in rs:
                    khs[nh % 2][pl.ds(r * 8, 8), :] = _lane_gather(k_s[g, pl.ds(r * 8, 8), :], idx)
            nv = voff[n_kt] // 8
            todo = [divmod(n, nv) for n in range(Dh * nv) if KP0 + n * KPS // (Dh * nv) == step]
            for d in sorted({d for d, _ in todo}):
                idx = jnp.where(keep[0], jnp.full((8, LANES), lo + d, i32), pltpu.bitcast(dep, i32))
                for r in [r for dd, r in todo if dd == d]:
                    kbs[nh % 2][0, d, pl.ds(r * 8, 8), :] = _lane_gather(kv_s[g, pl.ds(r * 8, 8), :], idx)
            un = u + 1
            hq = head(un)
            ds = [d for d in range(Dh) if QP0 + d * QPS // Dh == j]
            for half in sorted({d // 8 for d in ds}):
                qw = qf_s[un % n_qb + zero(u * n_kt + j), pl.ds(pl.multiple_of(hq * Dh + half * 8, 8), 8), :]
                for q in range(n_qt):
                    w = jnp.where(keep[0], qw[:, q * LANES:(q + 1) * LANES], dep)
                    for d in ds:
                        if d // 8 == half:
                            qbs[un % 2][0, d, :, pl.ds(q * LANES, LANES)] = jnp.broadcast_to(w[d % 8:d % 8 + 1], (8, LANES))

        probs = {blk: pend_s[pl.ds(n * 16, 16), :] for n, blk in enumerate(pending_in)}
        slot, done_tiles = 0, 0
        while slot < len(stream):
            kind, what = stream[slot]
            if kind == "k":
                u = what[0]
                end = slot
                while stream[end][0] == "k" and stream[end][1][0] == u:
                    end += 1
                lhs = [anchored(khs[(u // n_qb) % 2][pl.ds(stream[m][1][2] // 2, 8), :], m) for m in range(slot, end)]
                s = _dot(_unpack(jnp.concatenate(lhs, axis=0))[:, :Dh],
                         _unpack(q_rows(head(u), u % n_qb + zero(slot))))
                p = jnp.exp2(s)
                for n, m in enumerate(range(slot, end)):
                    probs[stream[m][1]] = p[n * 16:(n + 1) * 16]
                if slot == 0 or stream[slot - 1][0] == "v":
                    prep_piece(*divmod(done_tiles, n_kt), s[0:8, 0:LANES])
                slot = end
            else:
                u, j = what
                vt = v_rows(head(u), j * KC, KC)
                if PF32:
                    vt = jnp.concatenate([anchored(vt[0:8], slot), vt[8:16]], axis=0)
                else:
                    vt = anchored(vt, slot)
                l, acc = pv_tile(probs, partial, u, j, vt, l, acc)
                if j == n_kt - 1 or PVALL:
                    after[slot + PVD] = [acc[0:8, BQ - LANES:BQ]]
                if j == n_kt - 1:
                    finish(head(u), u % n_qb, l, acc)
                slot += 1
                done_tiles += 1
        for n, blk in enumerate(pending_out):
            pend_s[pl.ds(n * 16, 16), :] = probs.pop(blk)
        assert not assign and not probs and not partial
        return l, acc

    def fast_path():
        kb_b[0, :, pl.ds(voff[n_kt - 1], vk[n_kt - 1]), :] = jnp.zeros((Dh, vk[n_kt - 1], LANES), f32)
        qb_b[...] = jnp.zeros(qb_b.shape, f32)
        for n, (u, j, b) in enumerate(pending_in):
            if u < 0:
                pend_s[pl.ds(n * 16, 16), :] = jnp.zeros((16, BQ), f32)
            else:
                s = _dot(_unpack(kh_a[pl.ds(b // 2, 8), :])[:, :Dh], _unpack(q_rows(0, 0)))
                pend_s[pl.ds(n * 16, 16), :] = jnp.exp2(s)
        l, acc = lax.fori_loop(0, H // NH, fast_heads, (jnp.zeros((8, BQ), f32), jnp.zeros((Dh, BQ), f32)))
        u, j = tiles[-1]
        probs = {blk: pend_s[pl.ds(n * 16, 16), :] for n, blk in enumerate(pending_out) if blk[0] == u}
        partial = {}
        for pc in tile_pieces(j):
            run_piece(partial, u, j, pc, 0)
        l, acc = pv_tile(probs, partial, u, j, v_rows(H - 1, j * KC, KC), l, acc)
        finish(H - 1, n_qb - 1, l, acc)

    def guarded_item(it, _):
        h, qb = it // n_qb, it % n_qb

        @pl.when(qb == 0)
        def _():
            kh_a[...] = pltpu.roll(k_s[h // hpg], (LANES - (h % hpg) * Dh) % LANES, 1)

        qh = _unpack(q_rows(h, qb))
        step = 4 * KC

        def scores(c, m):
            r0 = pl.multiple_of(c * step, step)
            s = _dot(_unpack(kh_a[pl.ds(pl.multiple_of(r0 // 2, step // 2), step // 2), :])[:, :Dh], qh)
            s_s[pl.ds(r0, step), :] = s
            return functools.reduce(jnp.maximum, [m] + _rows8(s))

        m = lax.fori_loop(0, S // step, scores, jnp.full((8, BQ), -jnp.inf, f32))
        m = jnp.max(m, axis=0, keepdims=True)

        def values(c, carry):
            l, acc = carry
            r0 = pl.multiple_of(c * step, step)
            p = jnp.exp2(s_s[pl.ds(r0, step), :] - m)
            vt = v_rows(h, r0, step)
            pv = _dot(vt, p) if PF32 else _dot(_unpack(vt), p.astype(bf16))
            return functools.reduce(jnp.add, [l] + _rows8(p)), acc + pv

        l, acc = lax.fori_loop(0, S // step, values, (jnp.zeros((8, BQ), f32), jnp.zeros((Dh, BQ), f32)))
        finish(h, qb, l, acc)

    if ONLY in ("", "attn"):
        pl.when(safe)(fast_path)

    if ONLY == "":
        @pl.when(jnp.logical_not(safe))
        def _():
            lax.fori_loop(0, H * n_qb, guarded_item, None)

    F = w1_v.shape[1]
    b1 = b1_ref[pl.ds(0, F)].astype(f32).reshape(1, F)
    b2 = b2_ref[pl.ds(0, D)].astype(f32).reshape(1, D)
    out_cp = [pltpu.make_async_copy(out_v.at[pl.ds(r * RC, RC)], out_hbm.at[pl.ds(r * RC, RC)], out_sem.at[r])
              for r in range(n_rc)]

    def head_sums(ls):
        row = lax.broadcasted_iota(i32, ls[0].shape, 0)
        c = [jnp.where(row < 4, a, b) + pltpu.roll(jnp.where(row < 4, b, a), 4, 0) for a, b in zip(ls[:4], ls[4:])]
        for sh in (2, 1):
            low = (row & sh) == 0
            n = len(c) // 2
            c = [jnp.where(low, a, b) + jnp.where(low, pltpu.roll(a, 8 - sh, 0), pltpu.roll(b, sh, 0))
                 for a, b in zip(c[:n], c[n:])]
        return c[0]

    rh, dh, fh = RC // 2, D // 2, F // 2
    uses = ({0: 1, 3: 1}, {2: 1, 3: -1}, {1: 1, 3: 1}, {0: 1, 2: 1}, {0: -1, 1: 1}, {3: 1}, {0: 1})

    def combos(a11, a12, a21, a22):
        return a11 + a22, a21 + a22, a11, a22, a11 + a12, a21 - a11, a12 - a22

    def strassen(product, order):
        c = [None] * 4
        for n in order:
            m = product(n)
            for q, sign in uses[n].items():
                c[q] = (m if sign > 0 else -m) if c[q] is None else (c[q] + m if sign > 0 else c[q] - m)
        return c

    def normalize(r, h0, q, dep=None):
        cols = pl.ds(q * LANES, LANES)
        ls = [l_s[r, h, :, cols] for h in range(h0, h0 + 8)]
        inv = 1.0 / head_sums([held(ls[0], dep)] + ls[1:])
        ot = [ot_s[r, pl.ds((h0 + n) * Dh, Dh), cols] * inv[n:n + 1] for n in range(8)]
        o = jnp.concatenate(ot, axis=0).astype(bf16).T
        o_s[r][0, pl.ds(q * LANES // 2, LANES // 2), pl.ds(h0 * Dh, LANES)] = pltpu.bitcast(o, u32)

    def norm_jobs(r):
        return [functools.partial(normalize, r, h0, q) for q in range(n_qt) for h0 in range(0, H, 8)]

    def ffn_input(r, b, dep=None):
        top = _layernorm(held(h_s[r + zero0, pl.ds(b * 16, 16), :], dep))
        bot = _layernorm(held(h_s[r + zero0, pl.ds(rh + b * 16, 16), :], dep))
        for n, a in enumerate(combos(top[:, :dh], top[:, dh:], bot[:, :dh], bot[:, dh:])):
            a1_s[r][0, n, pl.ds(b * 8, 8), :] = _pack(a)

    def ln_jobs(r):
        return [functools.partial(ffn_input, r, b) for b in range(rh // 16)]

    def out_proj(r, todo):
        for g in range(n_g):
            cols = pl.ds(g * LANES, LANES)
            y = _dot(_unpack(o_s[r][g * zero0]), wo_v[:, cols])
            release(share(todo, g, OPG) if g < OPG else [], y)
            h_s[r, :, cols] = x_v[pl.ds(r * RC, RC), cols].astype(f32) + y

    def ffn(r, todo):
        for c0 in range(0, fh, LANES):
            cols = pl.ds(c0, LANES)
            u = strassen(lambda n: _dot(_unpack(a1_s[r][(c0 // LANES + 1) * zero0, n]), _unpack(w1t_s[n, :, cols])), ORD1)
            g = [_gelu2(u[q] + b1[:, (q % 2) * fh + c0:(q % 2) * fh + c0 + LANES]) for q in range(4)]
            for n, a in enumerate(combos(*g)):
                a2_s[n, :, cols] = _pack(a)

        def product(n):
            m = _dot(_unpack(a2_s[n]), _unpack(w2t_s[n]))
            i = ORD2.index(n)
            release(share(todo, i - RL0, RL1 - RL0) if RL0 <= i < RL1 else [], m)
            return m

        y = strassen(product, ORD2)
        for q in range(4):
            rows, cols = pl.ds((q // 2) * rh, rh), pl.ds((q % 2) * dh, dh)
            res = 0.5 * y[q] + b2[:, (q % 2) * dh:(q % 2 + 1) * dh] + h_s[r + zero0, rows, cols]
            out_v[pl.ds(r * RC + (q // 2) * rh, rh), cols] = res.astype(out_v.dtype)

    if ONLY in ("", "p2"):
        for fn in norm_jobs(0):
            fn()
        out_proj(0, norm_jobs(1))
        for r in range(n_rc):
            if r + 1 < n_rc:
                out_proj(r + 1, ln_jobs(0) if r == 0 else [])
            ffn(r, (norm_jobs(r + 2) if r + 2 < n_rc else []) + (ln_jobs(r + 1) if r + 1 < n_rc else []))
            out_cp[r].start()
    else:
        if ONLY == "p0":
            @pl.when(safe)
            def _():
                def bd(z, _):
                    z8 = pl.multiple_of(z * 8, 8)
                    out_v[0:16, 0:128] = (_unpack(kh_a[pl.ds(z8, 8), :]).astype(f32) + kb_a[0, z, 0:16, :] + qb_a[0, z, :, 0:128][0:1]
                                          + _unpack(k_s[z, 0:8, :]) + kv_s[z, 0:16, :] + _unpack(qt_s[z, 0:8, 0:128]) + qf_s[z, 0:16, 0:128]
                                          + _unpack(vt_s[pl.ds(z8, 8), 0:128]) + _unpack(w1t_s[z, 0:8, 0:128]) + _unpack(w2t_s[z, 0:8, 0:128])).astype(bf16)
                lax.fori_loop(0, 2, bd, None)
        for r in range(n_rc):
            out_v[pl.ds(r * RC + 16, 16), :] = (ot_s[r, 0:16, :] + l_s[r, 0:2].reshape(16, BQ)).astype(bf16)
            out_cp[r].start()
    for c in out_cp:
        c.wait()


@jax.jit
def pallas_sequential_preLN__softmax_full_mha__dense_activation_gelu__prompt_kernel(A_x, A_wqkv, A_wo, B_x, B_w1, B_b1, B_w2, B_b2):
    del B_x
    B, S, D = A_x.shape
    F = B_w1.shape[1]
    Dh = D // H
    n_rc = S // RC
    nvk = sum(VP[j % len(VP)] for j in range(S // KC))
    hbm = pl.BlockSpec(memory_space=pl.ANY)
    vmem = pl.BlockSpec(memory_space=pltpu.VMEM)
    V = pltpu.VMEM
    flags = None
    out = pl.pallas_call(
        _kernel,
        out_shape=jax.ShapeDtypeStruct((S, D), A_x.dtype),
        in_specs=[hbm] * 7,
        out_specs=hbm,
        scratch_shapes=[
            *([V((FRONT * 512,), B_b1.dtype)] if FRONT else []),
            V((S, D), A_x.dtype), V((3, D, D), bf16), V((D, D), bf16), V((D, F), bf16), V((F, D), bf16),
            V((D // 2, D), u32), V((D // 2, D), u32),
            *[V((1, RC // 2, D), u32) for _ in range(n_rc)],
            V((D // LANES, S // 2, LANES), u32),
            V((D // LANES, nvk, LANES), f32),
            V((S // BQ, D // 2, BQ), u32),
            V((S // BQ, D, BQ), f32),
            V((D, S), f32) if PF32 else V((D // 2, S), u32),
            V((S // BQ, D, BQ), f32),
            V((S // BQ, H, 8, BQ), f32),
            V((S // 2, LANES), u32), V((S // 2, LANES), u32),
            V((1, Dh, nvk, LANES), f32), V((1, Dh, nvk, LANES), f32),
            V((1, Dh, 8, BQ), f32), V((1, Dh, 8, BQ), f32),
            V((LAGB * 16, BQ), f32),
            V((S, BQ), f32),
            V((7, D // 4, F // 2), u32), V((7, F // 4, D // 2), u32),
            V((n_rc, RC, D), f32),
            *[V((1, RC // 2, D), u32) for _ in range(n_rc)],
            *[V((1, 7, RC // 4, D // 2), u32) for _ in range(n_rc)],
            V((7, RC // 4, F // 2), u32),
            V((S, D), A_x.dtype),
            pltpu.SMEM((4,), i32),
            pltpu.SemaphoreType.DMA((8 + n_rc,)),
            pltpu.SemaphoreType.DMA((n_rc,)),
            V((BACK * 512,), B_b2.dtype),
            *([] if FRONT else [V((2048,), B_b1.dtype)]),
        ],
        compiler_params=pltpu.CompilerParams(vmem_limit_bytes=100 * 1024 * 1024, flags=flags),
        name="fused_block",
    )(A_x.reshape(S, D), A_wqkv, A_wo, B_w1, B_b1, B_w2, B_b2)
    return out.reshape(B, S, D)
```

```python
import functools
import math

import jax
import jax.numpy as jnp
from jax import lax
import jax.experimental.pallas as pl
import jax.experimental.pallas.tpu as pltpu

H = 32
EPS = 1e-5
LANES = 128
RC = 512
BQ = 512
KC = 128
VPU_KEYS = (16, 16, 32, 16, 16, 16, 16, 32, 16, 16, 16, 16, 32, 16, 16, 16)
HEADS_PER_STEP = 2
LAG_BLOCKS = 8
SAFE_LOG2 = 80.0

f32 = jnp.float32
bf16 = jnp.bfloat16
u32 = jnp.uint32
i32 = jnp.int32


def _layernorm(x):
    m = jnp.mean(x, axis=-1, keepdims=True)
    xc = x - m
    v = jnp.mean(xc * xc, axis=-1, keepdims=True)
    return xc * lax.rsqrt(v + EPS)


def _gelu2(u):
    c0 = math.sqrt(2.0 / math.pi)
    c1 = c0 * 0.044715
    return u + u * jnp.tanh(u * (c0 + c1 * (u * u)))


def _rows8(x):
    return [x[i:i + 8] for i in range(0, x.shape[0], 8)]


def _pack(x):
    return pltpu.bitcast(x.astype(bf16), u32)


def _unpack(w):
    return pltpu.bitcast(w, bf16)


def _dot(a, b):
    return jnp.dot(a, b, preferred_element_type=f32)


def _dot_nt(a, b):
    return lax.dot_general(a, b, (((1,), (1,)), ((), ())), preferred_element_type=f32)


def _lane_gather(x, idx):
    return jnp.take_along_axis(x, idx, axis=1, mode="promise_in_bounds", wrap_negative_indices=False)


def _strassen_lhs(a11, a12, a21, a22):
    return a11 + a22, a21 + a22, a11, a22, a11 + a12, a21 - a11, a12 - a22


def _strassen_rhs(b11, b12, b21, b22):
    return b11 + b22, b11, b12 - b22, b21 - b11, b22, b11 + b12, b21 + b22


_STRASSEN_USES = (((0, 1), (3, 1)), ((2, 1), (3, -1)), ((1, 1), (3, 1)), ((0, 1), (2, 1)),
                  ((0, -1), (1, 1)), ((3, 1),), ((0, 1),))


def _strassen(product, order):
    c = [None] * 4
    for n in order:
        m = product(n)
        for q, sign in _STRASSEN_USES[n]:
            if c[q] is None:
                c[q] = (m, sign)
            elif c[q][1] == sign:
                c[q] = (c[q][0] + m, sign)
            else:
                c[q] = (m - c[q][0] if sign > 0 else c[q][0] - m, 1)
    assert all(sign > 0 for _, sign in c)
    return [v for v, _ in c]


def _row_sums8(xs):
    row = lax.broadcasted_iota(i32, xs[0].shape, 0)
    c = [jnp.where(row < 4, a, b) + pltpu.roll(jnp.where(row < 4, b, a), 4, 0)
         for a, b in zip(xs[:4], xs[4:])]
    for sh in (2, 1):
        low = (row & sh) == 0
        n = len(c) // 2
        c = [jnp.where(low, a, b) + jnp.where(low, pltpu.roll(a, 8 - sh, 0), pltpu.roll(b, sh, 0))
             for a, b in zip(c[:n], c[n:])]
    return c[0]


def _share(todo, n, parts):
    return todo[n * len(todo) // parts:(n + 1) * len(todo) // parts] if 0 <= n < parts else []


def _now(todo):
    for job in todo:
        job()


def _release(todo, y):
    vregs = [(t, c) for c in range(0, y.shape[1], LANES) for t in range(0, y.shape[0], 8)]
    for n, job in enumerate(todo):
        t, c = vregs[n * len(vregs) // len(todo)]
        job(y[t:t + 8, c:c + LANES])


def _block_kernel(x_hbm, wqkv_hbm, wo_hbm, w1_hbm, b1_hbm, w2_hbm, b2_hbm, out_hbm,
                  x_v, wqkv_v, wo_v, w1_v, w2_v, wqt_s, wvt_s, w1_t, w2_t,
                  xn_0, xn_1, xn_2, xn_3, k_s, kc_s, qt_s, qc_s, vt_s, ot_s, l_s,
                  kh_a, kh_b, kb_a, kb_b, qb_a, qb_b, pend_s, s_s,
                  ha_0, ha_1, ha_2, ha_3, h_s, ga_s, out_v, b1_v, b2_v, zero_s, in_sem, out_sem):
    S, D = x_v.shape
    F = w1_v.shape[1]
    Dh = D // H
    n_rc, n_qb, n_kt, n_qt, n_g = S // RC, S // BQ, S // KC, BQ // LANES, D // LANES
    hpg = LANES // Dh
    rh, dh, fh = RC // 2, D // 2, F // 2
    vk = VPU_KEYS
    voff = [sum(vk[:j]) for j in range(n_kt + 1)]
    xn_s = [xn_0, xn_1, xn_2, xn_3]
    ha_s = [ha_0, ha_1, ha_2, ha_3]

    def copy(src, dst, n):
        return pltpu.make_async_copy(src, dst, in_sem.at[n])

    wq_cp, wk_cp, wv_cp = (copy(wqkv_hbm.at[:, pl.ds(n * D, D)], wqkv_v.at[n], n) for n in range(3))
    ffn_cp = [copy(wo_hbm, wo_v, 3), copy(w1_hbm, w1_v, 4), copy(w2_hbm, w2_v, 5),
              copy(b1_hbm, b1_v.at[pl.ds(0, F)], 6), copy(b2_hbm, b2_v.at[pl.ds(0, D)], 7)]
    x_cp = [copy(x_hbm.at[pl.ds(r * RC, RC)], x_v.at[pl.ds(r * RC, RC)], 8 + r) for r in range(n_rc)]
    for c in x_cp[:1] + [wk_cp] + x_cp[1:] + [wq_cp, wv_cp] + ffn_cp:
        c.start()

    def put_zero(n, _):
        zero_s[n] = n // 65536

    lax.fori_loop(0, zero_s.shape[0], put_zero, None)
    zero = zero_s[0]
    keep = lax.broadcasted_iota(i32, (8, LANES), 0) >= zero

    def held(x, dep):
        if dep is None:
            return x
        head = jnp.concatenate([jnp.where(keep, t, dep) for t in _rows8(x[:, :LANES])], axis=0)
        return jnp.concatenate([head, x[:, LANES:]], axis=1) if x.shape[1] > LANES else head

    def weight_jobs(ref, table):
        kh, nh = ref.shape[0] // 2, ref.shape[1] // 2

        def job(t, c, dep):
            words = [pltpu.bitcast(ref[pl.ds(a * kh + t, 16), pl.ds(b * nh + c, LANES)], u32)
                     for a in range(2) for b in range(2)]
            words = [jnp.where(keep, w, pltpu.bitcast(dep, u32)) for w in words]
            blocks = [_unpack(w).astype(f32) for w in words]
            for n, b in enumerate(_strassen_rhs(*blocks)):
                same = [w for w, blk in zip(words, blocks) if blk is b]
                table[n, pl.ds(t // 2, 8), pl.ds(c, LANES)] = same[0] if same else _pack(b)

        return [functools.partial(job, t, c) for t in range(0, kh, 16) for c in range(0, nh, LANES)]

    peaks = {}

    def peak(name, w):
        peaks[name] = w if name not in peaks else jnp.maximum(peaks[name], w)

    def x_jobs(r, rows=32):
        def job(t, dep=None):
            xn = _layernorm(held(x_v[pl.ds(r * RC + t, rows), :].astype(f32), dep))
            xn_s[r][0, pl.ds(t // 2, rows // 2), :] = _pack(xn)

        return [functools.partial(job, t) for t in range(0, RC, rows)]

    k_squares, k_pairs = [], []

    def project_k(r, g, todo=()):
        k = _dot(_unpack(xn_s[r][g * zero]), wqkv_v[1, :, pl.ds(g * LANES, LANES)])
        _release(todo, k)
        k_s[g, pl.ds(r * RC // 2, RC // 2), :] = _pack(k)
        for t0 in range(0, RC, KC):
            j = (r * RC + t0) // KC
            for t in range(0, vk[j], 16):
                k_pairs.append((g, (voff[j] + t) // 2, k[t0 + t:t0 + t + 8], k[t0 + t + 8:t0 + t + 16]))
        k2 = _rows8(k * k)
        k_squares.extend(functools.reduce(jnp.maximum, k2[n:n + 8]) for n in range(0, len(k2), 8))

    def key_operands(g, row, a11, a21, dep):
        a11, a21 = held(a11, dep), held(a21, dep)
        a12, a22 = (pltpu.roll(a, LANES - Dh // 2, 1) for a in (a11, a21))
        s1 = a21 + a22
        s2 = s1 - a11
        for n, t in enumerate((a11, a12, a12 - s2, a22, s1, s2, a11 - a21)):
            kc_s[g, n, pl.ds(row, 8), :] = t

    def key_peak(w, dep):
        w = held(w, dep)
        for sh in (1, 2, 4, 8):
            w = w + pltpu.roll(w, sh, 1)
        peak("k", w)

    def first_tables(n, e, dep):
        kc = held(kc_s[0, n, pl.ds(0, voff[n_kt] // 2), :], dep)
        kb_a[0, n * 8 + e] = jnp.broadcast_to(kc[:, e:e + 1], kc.shape)
        qb_a[0, n * 8 + e] = jnp.broadcast_to(qc_s[0, 0, n, e:e + 1, :], (8, BQ // 2))

    def project_q(r, todo):
        qt = _dot_nt(_unpack(wqt_s[...]), _unpack(xn_s[r][0]))
        _release(todo, qt)
        qt = qt * ((Dh ** -0.5) * math.log2(math.e))
        qt_s[r] = _pack(qt)
        squares = []
        for h in range(H):
            lo, hi = _rows8(qt[h * Dh:(h + 1) * Dh])
            b11, b12, b21, b22 = (jnp.concatenate([t[:, c * LANES:(c + 1) * LANES] for c in (c0, c0 + 2)], axis=1)
                                  for t in (lo, hi) for c0 in range(2))
            t1 = b12 - b11
            t2 = b22 - t1
            for n, t in enumerate((b11, b21, b22, b21 - t2, t1, t2, b22 - b12)):
                qc_s[r, h, n] = t
            squares.append(lo * lo + hi * hi)
        for h0 in range(0, H, 8):
            peak("q", _row_sums8(squares[h0:h0 + 8]))

    def project_v(r, todo):
        vt = _dot_nt(_unpack(wvt_s[...]), _unpack(xn_s[r][0]))
        _release(todo, vt)
        vt_s[:, pl.ds(r * RC, RC)] = vt
        peak("v", functools.reduce(jnp.maximum, _rows8(jnp.abs(vt))))

    n_it = HEADS_PER_STEP * n_qb
    khs, kbs, qbs = [kh_a, kh_b], [kb_a, kb_b], [qb_a, qb_b]
    blocks = [(u, j, j * KC + b) for u in range(-1, n_it + 1) for j in range(n_kt)
              for b in range(KC - 16, vk[j] - 1, -16)]
    tile_end = {(u, j): n + 1 for n, (u, j, _) in enumerate(blocks)}
    tiles = [(-1, n_kt - 1)] + [(u, j) for u in range(n_it) for j in range(n_kt)]
    stream, n_streamed = [], tile_end[-1, n_kt - 2] + LAG_BLOCKS
    pending_in = blocks[tile_end[-1, n_kt - 2]:n_streamed]
    for tile in tiles[:-1]:
        stream += [("k", blk) for blk in blocks[n_streamed:tile_end[tile] + LAG_BLOCKS]] + [("v", tile)]
        n_streamed = tile_end[tile] + LAG_BLOCKS
    pending_out = blocks[tile_end[n_it - 1, n_kt - 2]:n_streamed]

    def q_rows(h, qb):
        return _unpack(qt_s[qb, pl.ds(pl.multiple_of(h * (Dh // 2), Dh // 2), Dh // 2), :])

    def start_stream():
        kb_b[0, :, pl.ds(voff[n_kt - 1] // 2, vk[-1] // 2), :] = jnp.zeros((56, vk[-1] // 2, LANES), f32)
        qb_b[...] = jnp.zeros(qb_b.shape, f32)
        for n, (u, _, b) in enumerate(pending_in):
            if u < 0:
                pend_s[pl.ds(n * 16, 16), :] = jnp.zeros((16, BQ), f32)
            else:
                s = _dot(_unpack(k_s[0, pl.ds(b // 2, 8), :])[:, :Dh], q_rows(0, 0))
                pend_s[pl.ds(n * 16, 16), :] = jnp.exp2(s)

    x_cp[0].wait()
    _now(x_jobs(0, RC))
    wk_cp.wait()
    for g in range(n_g - 1):
        project_k(0, g)
    x_cp[1].wait()
    todo = x_jobs(1)
    _now(todo[:4])
    project_k(0, n_g - 1, todo[4:])
    project_k(1, 0)
    project_k(1, 1)
    x_cp[2].wait()
    todo = x_jobs(2)
    _now(todo[:3])
    project_k(1, 2, todo[3:10])
    project_k(1, 3, todo[10:])
    project_k(2, 0)
    project_k(2, 1)
    x_cp[3].wait()
    wq_cp.wait()
    todo = x_jobs(3)
    _now(todo[:3])
    project_k(2, 2, todo[3:10])
    project_k(2, 3, todo[10:])
    wqt_s[...] = pltpu.bitcast(wqkv_v[0].T, u32)
    for g in range(n_g):
        project_k(3, g)
    project_q(0, [functools.partial(key_operands, *args) for args in sorted(k_pairs, key=lambda a: a[:2])])
    project_q(1, [functools.partial(key_peak, w) for w in k_squares])
    kh_a[...] = k_s[0]
    todo = [functools.partial(first_tables, n, e) for e in range(8) for n in range(7)]
    project_q(2, _share(todo, 0, 2))
    for c in [wv_cp] + ffn_cp:
        c.wait()
    wvt_s[...] = pltpu.bitcast(wqkv_v[2].T, u32)
    project_q(3, _share(todo, 1, 2))
    start_stream()
    todo = weight_jobs(w1_v, w1_t) + weight_jobs(w2_v, w2_t)
    for r in range(n_rc):
        project_v(r, _share(todo, r, n_rc))

    v_peak = jnp.max(peaks["v"])
    bounded = ((jnp.max(peaks["k"]) * jnp.max(peaks["q"]) <= SAFE_LOG2 * SAFE_LOG2)
               & (v_peak <= 2.0 ** 30) & (v_peak >= 2.0 ** -20))

    def v_rows(h, start, size):
        return vt_s[pl.ds(pl.multiple_of(h * Dh, Dh), Dh), pl.ds(start, size)]

    def finish(h, qb, l, acc):
        ot_s[qb, pl.ds(pl.multiple_of(h * Dh, Dh), Dh), :] = acc
        l_s[qb, h] = l

    def max_subtracting_item(it, _):
        h, qb = it // n_qb, it % n_qb

        @pl.when(qb == 0)
        def _():
            kh_a[...] = pltpu.roll(k_s[h // hpg], (LANES - (h % hpg) * Dh) % LANES, 1)

        qh = q_rows(h, qb)
        step = 4 * KC

        def scores(c, m):
            keys = kh_a[pl.ds(pl.multiple_of(c * (step // 2), step // 2), step // 2), :]
            s = _dot(_unpack(keys)[:, :Dh], qh)
            s_s[pl.ds(pl.multiple_of(c * step, step), step), :] = s
            return functools.reduce(jnp.maximum, [m] + _rows8(s))

        m = lax.fori_loop(0, S // step, scores, jnp.full((8, BQ), -jnp.inf, f32))
        m = jnp.max(m, axis=0, keepdims=True)

        def values(c, carry):
            l, acc = carry
            r0 = pl.multiple_of(c * step, step)
            p = jnp.exp2(s_s[pl.ds(r0, step), :] - m)
            return functools.reduce(jnp.add, [l] + _rows8(p)), acc + _dot(v_rows(h, r0, step), p)

        l, acc = lax.fori_loop(0, S // step, values, (jnp.zeros((8, BQ), f32), jnp.zeros((Dh, BQ), f32)))
        finish(h, qb, l, acc)

    def vpu_pieces(j):
        return [(t, n) for t in range(0, vk[j], 16) for n in range(7)]

    def vpu_piece(partial, u, j, piece, z):
        t, n = piece
        kb, qb = kbs[(u // n_qb) % 2], qbs[u % 2]
        a = partial.setdefault((u, j, t), {})
        marks = []

        def product(m, acc=None):
            for e in range(8):
                kk = kb[z, m * 8 + e, pl.ds((voff[j] + t) // 2, 8), :]
                term = jnp.concatenate([kk, kk], axis=1) * qb[z, m * 8 + e]
                acc = term if acc is None else acc + term
                if e == 5:
                    marks.extend([acc[:, :LANES], acc[:, LANES:]])
            return acc

        if n == 0:
            a["p1"] = product(0)
        elif n == 1:
            a["c11"] = product(1, a["p1"])
        elif n == 2:
            a["u2"] = product(5, a["p1"])
        elif n == 3:
            a["p5"] = product(4)
        elif n == 4:
            a["u3"] = product(6, a["u2"])
            a["u4"] = a["u2"] + a["p5"]
            a["c22"] = a["u3"] + a["p5"]
        elif n == 5:
            a["c12"] = product(2, a["u4"])
        else:
            a["c21"] = product(3, a["u3"])
        return marks

    def pv_tile(probs, partial, u, j, vt, l, acc):
        rows = []
        for t in range(0, vk[j], 16):
            a = partial.pop((u, j, t))
            for names in (("c11", "c12"), ("c21", "c22")):
                s = jnp.concatenate([a[name][:, c:c + LANES] for c in (0, LANES) for name in names], axis=1)
                rows.append(jnp.exp2(s))
        rows += [probs.pop((u, j, j * KC + b)) for b in range(vk[j], KC, 16)]
        p = jnp.concatenate(rows, axis=0)
        l = functools.reduce(jnp.add, ([] if j == 0 else [l]) + _rows8(p)[::-1])
        pv = _dot(vt, p)
        return l, (pv if j == 0 else acc + pv)

    def bounded_heads(i, carry):
        l, acc = carry
        row = lax.broadcasted_iota(i32, (8, LANES), 0)
        lane = lax.broadcasted_iota(i32, (8, LANES), 1)
        keeps = [row > (i // 65536 - 1 - a) for a in range(3)]

        def nought(t):
            return (i * 4096 + t) // (4096 * H)

        def head(u):
            return jnp.clip(HEADS_PER_STEP * i + u // n_qb, 0, H - 1)

        pieces = [(u, j, pc) for (u, j) in tiles[:-1] for pc in vpu_pieces(j)]
        pv_slot = {what: n for n, (kind, what) in enumerate(stream) if kind == "v"}
        placed, after, partial = {}, {}, {}
        for n, pc in enumerate(pieces):
            slot = int((n + 1) * len(stream) / len(pieces) - 3.5)
            placed.setdefault(max(2, min(slot, pv_slot[pc[:2]])), []).append(pc)

        def anchored(x, slot):
            deps = []
            for (u, j, pc) in placed.pop(slot, []):
                deps = vpu_piece(partial, u, j, pc, nought((u + 1) * n_kt + j))
            for mask, dep in zip(keeps, deps + after.pop(slot, [])):
                x = jnp.where(mask, x, dep if x.dtype == f32 else pltpu.bitcast(dep, u32))
            return x

        def prepare(u, j, dep):
            nh = u // n_qb + 1
            hn = head(nh * n_qb)
            g, lo = hn // hpg, (hn % hpg) * Dh
            step = (u % n_qb) * n_kt + j - 1
            rs = _share([b // 16 for (uu, _, b) in blocks if uu == 0], step, 58)
            if rs:
                idx = jnp.where(keeps[0], (lane + lo) & (LANES - 1), pltpu.bitcast(dep, i32))
                for r in rs:
                    khs[nh % 2][pl.ds(r * 8, 8), :] = _lane_gather(k_s[g, pl.ds(r * 8, 8), :], idx)
            cells = [(e, n, r) for e in range(8) for n in range(7) for r in range(voff[n_kt] // 16)]
            cells = _share(cells, step, 58)
            for e in sorted({c[0] for c in cells}):
                idx = jnp.where(keeps[0], jnp.full((8, LANES), lo + e, i32), pltpu.bitcast(dep, i32))
                for (_, n, r) in [c for c in cells if c[0] == e]:
                    kbs[nh % 2][0, n * 8 + e, pl.ds(r * 8, 8), :] = _lane_gather(kc_s[g, n, pl.ds(r * 8, 8), :], idx)
            for m in _share(list(range(14)), j - 1, 14):
                n, cols = m // 2, pl.ds((m % 2) * LANES, LANES)
                w = jnp.where(keeps[0], qc_s[(u + 1) % n_qb, head(u + 1), n, :, cols], dep)
                for e in range(8):
                    qbs[(u + 1) % 2][0, n * 8 + e, :, cols] = jnp.broadcast_to(w[e:e + 1], (8, LANES))

        probs = {blk: pend_s[pl.ds(n * 16, 16), :] for n, blk in enumerate(pending_in)}
        slot = done = 0
        while slot < len(stream):
            kind, what = stream[slot]
            if kind == "k":
                u, end = what[0], slot
                while stream[end][0] == "k" and stream[end][1][0] == u:
                    end += 1
                keys = [anchored(khs[(u // n_qb) % 2][pl.ds(stream[m][1][2] // 2, 8), :], m)
                        for m in range(slot, end)]
                s = _dot(_unpack(jnp.concatenate(keys, axis=0))[:, :Dh], q_rows(head(u), u % n_qb + nought(slot)))
                p = jnp.exp2(s)
                for n, m in enumerate(range(slot, end)):
                    probs[stream[m][1]] = p[n * 16:(n + 1) * 16]
                if slot == 0 or stream[slot - 1][0] == "v":
                    prepare(*divmod(done, n_kt), s[0:8, 0:LANES])
                slot = end
            else:
                u, j = what
                vt = v_rows(head(u), j * KC, KC)
                vt = jnp.concatenate([anchored(vt[0:8], slot), vt[8:16]], axis=0)
                l, acc = pv_tile(probs, partial, u, j, vt, l, acc)
                after[slot + 10] = [acc[0:8, BQ - LANES:BQ]]
                if j == n_kt - 1:
                    finish(head(u), u % n_qb, l, acc)
                slot += 1
                done += 1
        for n, blk in enumerate(pending_out):
            pend_s[pl.ds(n * 16, 16), :] = probs.pop(blk)
        assert not placed and not probs and not partial
        return l, acc

    @pl.when(bounded)
    def _():
        l, acc = lax.fori_loop(0, H // HEADS_PER_STEP, bounded_heads,
                               (jnp.zeros((8, BQ), f32), jnp.zeros((Dh, BQ), f32)))
        u, j = tiles[-1]
        probs = {blk: pend_s[pl.ds(n * 16, 16), :] for n, blk in enumerate(pending_out) if blk[0] == u}
        partial = {}
        for pc in vpu_pieces(j):
            vpu_piece(partial, u, j, pc, 0)
        l, acc = pv_tile(probs, partial, u, j, v_rows(H - 1, j * KC, KC), l, acc)
        finish(H - 1, n_qb - 1, l, acc)

    @pl.when(jnp.logical_not(bounded))
    def _():
        lax.fori_loop(0, H * n_qb, max_subtracting_item, None)

    b1 = b1_v[pl.ds(0, F)].astype(f32).reshape(1, F)
    b2 = b2_v[pl.ds(0, D)].astype(f32).reshape(1, D)
    out_cp = [pltpu.make_async_copy(out_v.at[pl.ds(n * rh, rh)], out_hbm.at[pl.ds(n * rh, rh)], out_sem.at[n])
              for n in range(2 * n_rc)]

    def o_jobs(r):
        def job(h0, q, dep=None):
            cols = pl.ds(q * LANES, LANES)
            ls = [l_s[r, h, :, cols] for h in range(h0, h0 + 8)]
            inv = 1.0 / _row_sums8([held(ls[0], dep)] + ls[1:])
            ot = [ot_s[r, pl.ds((h0 + n) * Dh, Dh), cols] * inv[n:n + 1] for n in range(8)]
            o = jnp.concatenate(ot, axis=0).astype(bf16).T
            xn_s[r][0, pl.ds(q * LANES // 2, LANES // 2), pl.ds(h0 * Dh, LANES)] = pltpu.bitcast(o, u32)

        return [functools.partial(job, h0, q) for q in range(n_qt) for h0 in range(0, H, 8)]

    def h_jobs(r):
        def job(t, dep):
            top, bot = (_layernorm(held(h_s[r + zero, pl.ds(r0, 16), :], dep)) for r0 in (t, rh + t))
            for n, a in enumerate(_strassen_lhs(top[:, :dh], top[:, dh:], bot[:, :dh], bot[:, dh:])):
                ha_s[r][0, n, pl.ds(t // 2, 8), :] = _pack(a)

        return [functools.partial(job, t) for t in range(0, rh, 16)]

    def out_proj(r, todo):
        for g in range(n_g):
            cols = pl.ds(g * LANES, LANES)
            y = _dot(_unpack(xn_s[r][g * zero]), wo_v[:, cols])
            _release(_share(todo, g, n_g - 1), y)
            h_s[r, :, cols] = x_v[pl.ds(r * RC, RC), cols].astype(f32) + y

    def ffn(r, todo):
        for c in range(0, fh, LANES):
            cols = pl.ds(c, LANES)
            u = _strassen(lambda n: _dot(_unpack(ha_s[r][(c // LANES + 1) * zero, n]), _unpack(w1_t[n, :, cols])),
                          (2, 4, 5, 1, 0, 3, 6))
            g = [_gelu2(u[q] + b1[:, (q % 2) * fh + c:(q % 2) * fh + c + LANES]) for q in range(4)]
            for n, a in enumerate(_strassen_lhs(*g)):
                ga_s[n, :, cols] = _pack(a)
        order = (2, 5, 0, 4, 1, 6, 3) if r + 1 < n_rc else (2, 5, 0, 1, 3, 4, 6)

        def product(n):
            m = _dot(_unpack(ga_s[n]), _unpack(w2_t[n]))
            _release(_share(todo, order.index(n), 6), m)
            return m

        y = _strassen(product, order)
        for q in (2, 3, 0, 1):
            r0, cols = (q // 2) * rh, pl.ds((q % 2) * dh, dh)
            res = 0.5 * y[q] + b2[:, (q % 2) * dh:(q % 2 + 1) * dh] + h_s[r + zero, pl.ds(r0, rh), cols]
            out_v[pl.ds(r * RC + r0, rh), cols] = res.astype(out_v.dtype)
            if q % 2:
                out_cp[2 * r + q // 2].start()

    _now(o_jobs(0))
    out_proj(0, o_jobs(1))
    for r in range(n_rc):
        if r + 1 < n_rc:
            out_proj(r + 1, h_jobs(0) if r == 0 else [])
        ffn(r, (o_jobs(r + 2) if r + 2 < n_rc else []) + (h_jobs(r + 1) if r + 1 < n_rc else []))
    for c in out_cp:
        c.wait()


@jax.jit
def pallas_sequential_preLN__softmax_full_mha__dense_activation_gelu__prompt_kernel(
    A_x: jax.Array,
    A_wqkv: jax.Array,
    A_wo: jax.Array,
    B_x: jax.Array,
    B_w1: jax.Array,
    B_b1: jax.Array,
    B_w2: jax.Array,
    B_b2: jax.Array,
):
    del B_x
    B, S, D = A_x.shape
    F = B_w1.shape[1]
    n_rc = S // RC
    assert (B, n_rc, S // KC, D // H, RC) == (1, 4, len(VPU_KEYS), 16, BQ)
    pairs = sum(VPU_KEYS) // 16
    V = pltpu.VMEM
    scratch = [
        V((S, D), A_x.dtype), V((3, D, D), A_wqkv.dtype), V((D, D), A_wo.dtype),
        V((D, F), B_w1.dtype), V((F, D), B_w2.dtype),
        V((D // 2, D), u32), V((D // 2, D), u32),
        V((7, D // 4, F // 2), u32), V((7, F // 4, D // 2), u32),
        *[V((1, RC // 2, D), u32) for _ in range(n_rc)],
        V((D // LANES, S // 2, LANES), u32),
        V((D // LANES, 7, -(-pairs // 4) * 32, LANES), f32),
        V((S // BQ, D // 2, BQ), u32),
        V((S // BQ, H, 8, 8, BQ // 2), f32),
        V((D, S), f32),
        V((S // BQ, D, BQ), f32),
        V((S // BQ, H, 8, BQ), f32),
        V((S // 2, LANES), u32), V((S // 2, LANES), u32),
        V((1, 56, pairs * 8, LANES), f32), V((1, 56, pairs * 8, LANES), f32),
        V((1, 56, 8, BQ // 2), f32), V((1, 56, 8, BQ // 2), f32),
        V((LAG_BLOCKS * 16, BQ), f32),
        V((S, BQ), f32),
        *[V((1, 7, RC // 4, D // 2), u32) for _ in range(n_rc)],
        V((n_rc, RC, D), f32),
        V((7, RC // 4, F // 2), u32),
        V((S, D), A_x.dtype),
        V((2048,), B_b1.dtype), V((2048,), B_b2.dtype),
        pltpu.SMEM((4,), i32),
        pltpu.SemaphoreType.DMA((8 + n_rc,)),
        pltpu.SemaphoreType.DMA((2 * n_rc,)),
    ]
    hbm = pl.BlockSpec(memory_space=pl.ANY)
    out = pl.pallas_call(
        _block_kernel,
        out_shape=jax.ShapeDtypeStruct((S, D), A_x.dtype),
        in_specs=[hbm] * 7,
        out_specs=hbm,
        scratch_shapes=scratch,
        compiler_params=pltpu.CompilerParams(vmem_limit_bytes=100 * 1024 * 1024),
        name="fused_block",
    )(A_x.reshape(S, D), A_wqkv, A_wo, B_w1, B_b1, B_w2, B_b2)
    return out.reshape(B, S, D)
```

```python
import functools
import math

import jax
import jax.numpy as jnp
from jax import lax
import jax.experimental.pallas as pl
import jax.experimental.pallas.tpu as pltpu

H = 32
EPS = 1e-5
LANES = 128
RC = 512
BQ = 512
KC = 128
VPU_KEYS = (16, 16, 32, 16, 16, 16, 16, 32, 16, 16, 16, 16, 32, 16, 16, 16)
HEADS_PER_STEP = 2
LAG_BLOCKS = 8
SAFE_LOG2 = 80.0

f32 = jnp.float32
bf16 = jnp.bfloat16
u32 = jnp.uint32
i32 = jnp.int32


def _layernorm(x):
    m = jnp.mean(x, axis=-1, keepdims=True)
    xc = x - m
    v = jnp.mean(xc * xc, axis=-1, keepdims=True)
    return xc * lax.rsqrt(v + EPS)


def _gelu2(u):
    c0 = math.sqrt(2.0 / math.pi)
    c1 = c0 * 0.044715
    return u + u * jnp.tanh(u * (c0 + c1 * (u * u)))


def _rows8(x):
    return [x[i:i + 8] for i in range(0, x.shape[0], 8)]


def _pack(x):
    return pltpu.bitcast(x.astype(bf16), u32)


def _unpack(w):
    return pltpu.bitcast(w, bf16)


def _dot(a, b):
    return jnp.dot(a, b, preferred_element_type=f32)


def _dot_nt(a, b):
    return lax.dot_general(a, b, (((1,), (1,)), ((), ())), preferred_element_type=f32)


def _lane_gather(x, idx):
    return jnp.take_along_axis(x, idx, axis=1, mode="promise_in_bounds", wrap_negative_indices=False)


def _strassen_lhs(a11, a12, a21, a22):
    return a11 + a22, a21 + a22, a11, a22, a11 + a12, a21 - a11, a12 - a22


def _strassen_rhs(b11, b12, b21, b22):
    return b11 + b22, b11, b12 - b22, b21 - b11, b22, b11 + b12, b21 + b22


_STRASSEN_USES = (((0, 1), (3, 1)), ((2, 1), (3, -1)), ((1, 1), (3, 1)), ((0, 1), (2, 1)),
                  ((0, -1), (1, 1)), ((3, 1),), ((0, 1),))


def _strassen(product, order):
    c = [None] * 4
    for n in order:
        m = product(n)
        for q, sign in _STRASSEN_USES[n]:
            if c[q] is None:
                c[q] = (m, sign)
            elif c[q][1] == sign:
                c[q] = (c[q][0] + m, sign)
            else:
                c[q] = (m - c[q][0] if sign > 0 else c[q][0] - m, 1)
    assert all(sign > 0 for _, sign in c)
    return [v for v, _ in c]


def _row_sums8(xs):
    row = lax.broadcasted_iota(i32, xs[0].shape, 0)
    c = [jnp.where(row < 4, a, b) + pltpu.roll(jnp.where(row < 4, b, a), 4, 0)
         for a, b in zip(xs[:4], xs[4:])]
    for sh in (2, 1):
        low = (row & sh) == 0
        n = len(c) // 2
        c = [jnp.where(low, a, b) + jnp.where(low, pltpu.roll(a, 8 - sh, 0), pltpu.roll(b, sh, 0))
             for a, b in zip(c[:n], c[n:])]
    return c[0]


def _share(todo, n, parts):
    return todo[n * len(todo) // parts:(n + 1) * len(todo) // parts] if 0 <= n < parts else []


def _now(todo):
    for job in todo:
        job()


def _release(todo, y):
    vregs = [(t, c) for c in range(0, y.shape[1], LANES) for t in range(0, y.shape[0], 8)]
    for n, job in enumerate(todo):
        t, c = vregs[n * len(vregs) // len(todo)]
        job(y[t:t + 8, c:c + LANES])


def _block_kernel(x_hbm, wqkv_hbm, wo_hbm, w1_hbm, b1_hbm, w2_hbm, b2_hbm, out_hbm,
                  x_v, wqkv_v, wo_v, w1_v, w2_v, wqt_s, wvt_s, w1_t, w2_t,
                  xn_0, xn_1, xn_2, xn_3, k_s, kc_s, qt_s, qc_s, vt_s, ot_s, l_s,
                  kh_a, kh_b, kb_a, kb_b, qb_a, qb_b, pend_s, s_s,
                  ha_0, ha_1, ha_2, ha_3, h_s, ga_s, out_v, b1_v, b2_v, zero_s, in_sem, out_sem):
    S, D = x_v.shape
    F = w1_v.shape[1]
    Dh = D // H
    n_rc, n_qb, n_kt, n_qt, n_g = S // RC, S // BQ, S // KC, BQ // LANES, D // LANES
    hpg = LANES // Dh
    rh, dh, fh = RC // 2, D // 2, F // 2
    vk = VPU_KEYS
    voff = [sum(vk[:j]) for j in range(n_kt + 1)]
    xn_s = [xn_0, xn_1, xn_2, xn_3]
    ha_s = [ha_0, ha_1, ha_2, ha_3]

    def copy(src, dst, n):
        return pltpu.make_async_copy(src, dst, in_sem.at[n])

    wq_cp, wk_cp, wv_cp = (copy(wqkv_hbm.at[:, pl.ds(n * D, D)], wqkv_v.at[n], n) for n in range(3))
    ffn_cp = [copy(wo_hbm, wo_v, 3), copy(w1_hbm, w1_v, 4), copy(w2_hbm, w2_v, 5),
              copy(b1_hbm, b1_v.at[pl.ds(0, F)], 6), copy(b2_hbm, b2_v.at[pl.ds(0, D)], 7)]
    x_cp = [copy(x_hbm.at[pl.ds(r * RC, RC)], x_v.at[pl.ds(r * RC, RC)], 8 + r) for r in range(n_rc)]
    for c in x_cp[:1] + [wk_cp] + x_cp[1:] + [wq_cp, wv_cp] + ffn_cp:
        c.start()

    def put_zero(n, _):
        zero_s[n] = n // 65536

    lax.fori_loop(0, zero_s.shape[0], put_zero, None)
    zero = zero_s[0]
    keep = lax.broadcasted_iota(i32, (8, LANES), 0) >= zero

    def held(x, dep):
        if dep is None:
            return x
        head = jnp.concatenate([jnp.where(keep, t, dep) for t in _rows8(x[:, :LANES])], axis=0)
        return jnp.concatenate([head, x[:, LANES:]], axis=1) if x.shape[1] > LANES else head

    def weight_jobs(ref, table):
        kh, nh = ref.shape[0] // 2, ref.shape[1] // 2

        def job(t, c, dep):
            words = [pltpu.bitcast(ref[pl.ds(a * kh + t, 16), pl.ds(b * nh + c, LANES)], u32)
                     for a in range(2) for b in range(2)]
            words = [jnp.where(keep, w, pltpu.bitcast(dep, u32)) for w in words]
            blocks = [_unpack(w).astype(f32) for w in words]
            for n, b in enumerate(_strassen_rhs(*blocks)):
                same = [w for w, blk in zip(words, blocks) if blk is b]
                table[n, pl.ds(t // 2, 8), pl.ds(c, LANES)] = same[0] if same else _pack(b)

        return [functools.partial(job, t, c) for t in range(0, kh, 16) for c in range(0, nh, LANES)]

    peaks = {}

    def peak(name, w):
        peaks[name] = w if name not in peaks else jnp.maximum(peaks[name], w)

    def x_jobs(r, rows=32):
        def job(t, dep=None):
            xn = _layernorm(held(x_v[pl.ds(r * RC + t, rows), :].astype(f32), dep))
            xn_s[r][0, pl.ds(t // 2, rows // 2), :] = _pack(xn)

        return [functools.partial(job, t) for t in range(0, RC, rows)]

    k_squares, k_pairs = [], []

    def project_k(r, g, todo=()):
        k = _dot(_unpack(xn_s[r][g * zero]), wqkv_v[1, :, pl.ds(g * LANES, LANES)])
        _release(todo, k)
        k_s[g, pl.ds(r * RC // 2, RC // 2), :] = _pack(k)
        for t0 in range(0, RC, KC):
            j = (r * RC + t0) // KC
            for t in range(0, vk[j], 16):
                k_pairs.append((g, (voff[j] + t) // 2, k[t0 + t:t0 + t + 8], k[t0 + t + 8:t0 + t + 16]))
        k2 = _rows8(k * k)
        k_squares.extend(functools.reduce(jnp.maximum, k2[n:n + 8]) for n in range(0, len(k2), 8))

    def key_operands(g, row, a11, a21, dep):
        a11, a21 = held(a11, dep), held(a21, dep)
        a12, a22 = (pltpu.roll(a, LANES - Dh // 2, 1) for a in (a11, a21))
        s1 = a21 + a22
        s2 = s1 - a11
        for n, t in enumerate((a11, a12, a12 - s2, a22, s1, s2, a11 - a21)):
            kc_s[g, n, pl.ds(row, 8), :] = t

    def key_peak(w, dep):
        w = held(w, dep)
        for sh in (1, 2, 4, 8):
            w = w + pltpu.roll(w, sh, 1)
        peak("k", w)

    def first_tables(n, e, dep):
        kc = held(kc_s[0, n, pl.ds(0, voff[n_kt] // 2), :], dep)
        kb_a[0, n * 8 + e] = jnp.broadcast_to(kc[:, e:e + 1], kc.shape)
        qb_a[0, n * 8 + e] = jnp.broadcast_to(qc_s[0, 0, n, e:e + 1, :], (8, BQ // 2))

    def project_q(r, todo):
        qt = _dot_nt(_unpack(wqt_s[...]), _unpack(xn_s[r][0]))
        _release(todo, qt)
        qt = qt * ((Dh ** -0.5) * math.log2(math.e))
        qt_s[r] = _pack(qt)
        squares = []
        for h in range(H):
            lo, hi = _rows8(qt[h * Dh:(h + 1) * Dh])
            b11, b12, b21, b22 = (jnp.concatenate([t[:, c * LANES:(c + 1) * LANES] for c in (c0, c0 + 2)], axis=1)
                                  for t in (lo, hi) for c0 in range(2))
            t1 = b12 - b11
            t2 = b22 - t1
            for n, t in enumerate((b11, b21, b22, b21 - t2, t1, t2, b22 - b12)):
                qc_s[r, h, n] = t
            squares.append(lo * lo + hi * hi)
        for h0 in range(0, H, 8):
            peak("q", _row_sums8(squares[h0:h0 + 8]))

    def project_v(r, todo):
        vt = _dot_nt(_unpack(wvt_s[...]), _unpack(xn_s[r][0]))
        _release(todo, vt)
        vt_s[:, pl.ds(r * RC, RC)] = vt
        peak("v", functools.reduce(jnp.maximum, _rows8(jnp.abs(vt))))

    n_it = HEADS_PER_STEP * n_qb
    khs, kbs, qbs = [kh_a, kh_b], [kb_a, kb_b], [qb_a, qb_b]
    blocks = [(u, j, j * KC + b) for u in range(-1, n_it + 1) for j in range(n_kt)
              for b in range(KC - 16, vk[j] - 1, -16)]
    tile_end = {(u, j): n + 1 for n, (u, j, _) in enumerate(blocks)}
    tiles = [(-1, n_kt - 1)] + [(u, j) for u in range(n_it) for j in range(n_kt)]
    stream, n_streamed = [], tile_end[-1, n_kt - 2] + LAG_BLOCKS
    pending_in = blocks[tile_end[-1, n_kt - 2]:n_streamed]
    for tile in tiles[:-1]:
        stream += [("k", blk) for blk in blocks[n_streamed:tile_end[tile] + LAG_BLOCKS]] + [("v", tile)]
        n_streamed = tile_end[tile] + LAG_BLOCKS
    pending_out = blocks[tile_end[n_it - 1, n_kt - 2]:n_streamed]

    def q_rows(h, qb):
        return _unpack(qt_s[qb, pl.ds(pl.multiple_of(h * (Dh // 2), Dh // 2), Dh // 2), :])

    def start_stream():
        kb_b[0, :, pl.ds(voff[n_kt - 1] // 2, vk[-1] // 2), :] = jnp.zeros((56, vk[-1] // 2, LANES), f32)
        qb_b[...] = jnp.zeros(qb_b.shape, f32)
        for n, (u, _, b) in enumerate(pending_in):
            if u < 0:
                pend_s[pl.ds(n * 16, 16), :] = jnp.zeros((16, BQ), f32)
            else:
                s = _dot(_unpack(k_s[0, pl.ds(b // 2, 8), :])[:, :Dh], q_rows(0, 0))
                pend_s[pl.ds(n * 16, 16), :] = jnp.exp2(s)

    x_cp[0].wait()
    _now(x_jobs(0, RC))
    wk_cp.wait()
    project_k(0, 0)
    project_k(0, 1)
    x_cp[1].wait()
    todo = x_jobs(1)
    _now(todo[:3])
    project_k(0, 2, todo[3:10])
    project_k(0, 3, todo[10:])
    project_k(1, 0)
    project_k(1, 1)
    x_cp[2].wait()
    todo = x_jobs(2)
    _now(todo[:3])
    project_k(1, 2, todo[3:10])
    project_k(1, 3, todo[10:])
    project_k(2, 0)
    project_k(2, 1)
    x_cp[3].wait()
    wq_cp.wait()
    todo = x_jobs(3)
    _now(todo[:3])
    project_k(2, 2, todo[3:10])
    project_k(2, 3, todo[10:])
    wqt_s[...] = pltpu.bitcast(wqkv_v[0].T, u32)
    for g in range(n_g):
        project_k(3, g)
    project_q(0, [functools.partial(key_operands, *args) for args in sorted(k_pairs, key=lambda a: a[:2])])
    project_q(1, [functools.partial(key_peak, w) for w in k_squares])
    kh_a[...] = k_s[0]
    todo = [functools.partial(first_tables, n, e) for e in range(8) for n in range(7)]
    project_q(2, _share(todo, 0, 2))
    for c in [wv_cp] + ffn_cp:
        c.wait()
    wvt_s[...] = pltpu.bitcast(wqkv_v[2].T, u32)
    project_q(3, _share(todo, 1, 2))
    start_stream()
    todo = weight_jobs(w1_v, w1_t) + weight_jobs(w2_v, w2_t)
    for r in range(n_rc):
        project_v(r, _share(todo, r, n_rc))

    v_peak = jnp.max(peaks["v"])
    bounded = ((jnp.max(peaks["k"]) * jnp.max(peaks["q"]) <= SAFE_LOG2 * SAFE_LOG2)
               & (v_peak <= 2.0 ** 30) & (v_peak >= 2.0 ** -20))

    def v_rows(h, start, size):
        return vt_s[pl.ds(pl.multiple_of(h * Dh, Dh), Dh), pl.ds(start, size)]

    def finish(h, qb, l, acc):
        ot_s[qb, pl.ds(pl.multiple_of(h * Dh, Dh), Dh), :] = acc
        l_s[qb, h] = l

    def max_subtracting_item(it, _):
        h, qb = it // n_qb, it % n_qb

        @pl.when(qb == 0)
        def _():
            kh_a[...] = pltpu.roll(k_s[h // hpg], (LANES - (h % hpg) * Dh) % LANES, 1)

        qh = q_rows(h, qb)
        step = 4 * KC

        def scores(c, m):
            keys = kh_a[pl.ds(pl.multiple_of(c * (step // 2), step // 2), step // 2), :]
            s = _dot(_unpack(keys)[:, :Dh], qh)
            s_s[pl.ds(pl.multiple_of(c * step, step), step), :] = s
            return functools.reduce(jnp.maximum, [m] + _rows8(s))

        m = lax.fori_loop(0, S // step, scores, jnp.full((8, BQ), -jnp.inf, f32))
        m = jnp.max(m, axis=0, keepdims=True)

        def values(c, carry):
            l, acc = carry
            r0 = pl.multiple_of(c * step, step)
            p = jnp.exp2(s_s[pl.ds(r0, step), :] - m)
            return functools.reduce(jnp.add, [l] + _rows8(p)), acc + _dot(v_rows(h, r0, step), p)

        l, acc = lax.fori_loop(0, S // step, values, (jnp.zeros((8, BQ), f32), jnp.zeros((Dh, BQ), f32)))
        finish(h, qb, l, acc)

    def vpu_pieces(j):
        return [(t, n) for t in range(0, vk[j], 16) for n in range(7)]

    def vpu_piece(partial, u, j, piece, z):
        t, n = piece
        kb, qb = kbs[(u // n_qb) % 2], qbs[u % 2]
        a = partial.setdefault((u, j, t), {})
        marks = []

        def product(m, acc=None):
            for e in range(8):
                kk = kb[z, m * 8 + e, pl.ds((voff[j] + t) // 2, 8), :]
                term = jnp.concatenate([kk, kk], axis=1) * qb[z, m * 8 + e]
                acc = term if acc is None else acc + term
                if e == 5:
                    marks.extend([acc[:, :LANES], acc[:, LANES:]])
            return acc

        if n == 0:
            a["p1"] = product(0)
        elif n == 1:
            a["c11"] = product(1, a["p1"])
        elif n == 2:
            a["u2"] = product(5, a["p1"])
        elif n == 3:
            a["p5"] = product(4)
        elif n == 4:
            a["u3"] = product(6, a["u2"])
            a["u4"] = a["u2"] + a["p5"]
            a["c22"] = a["u3"] + a["p5"]
        elif n == 5:
            a["c12"] = product(2, a["u4"])
        else:
            a["c21"] = product(3, a["u3"])
        return marks

    def pv_tile(probs, partial, u, j, vt, l, acc):
        rows = []
        for t in range(0, vk[j], 16):
            a = partial.pop((u, j, t))
            for names in (("c11", "c12"), ("c21", "c22")):
                s = jnp.concatenate([a[name][:, c:c + LANES] for c in (0, LANES) for name in names], axis=1)
                rows.append(jnp.exp2(s))
        rows += [probs.pop((u, j, j * KC + b)) for b in range(vk[j], KC, 16)]
        p = jnp.concatenate(rows, axis=0)
        l = functools.reduce(jnp.add, ([] if j == 0 else [l]) + _rows8(p)[::-1])
        pv = _dot(vt, p)
        return l, (pv if j == 0 else acc + pv)

    def bounded_heads(i, carry):
        l, acc = carry
        row = lax.broadcasted_iota(i32, (8, LANES), 0)
        lane = lax.broadcasted_iota(i32, (8, LANES), 1)
        keeps = [row > (i // 65536 - 1 - a) for a in range(3)]

        def nought(t):
            return (i * 4096 + t) // (4096 * H)

        def head(u):
            return jnp.clip(HEADS_PER_STEP * i + u // n_qb, 0, H - 1)

        pieces = [(u, j, pc) for (u, j) in tiles[:-1] for pc in vpu_pieces(j)]
        pv_slot = {what: n for n, (kind, what) in enumerate(stream) if kind == "v"}
        placed, after, partial = {}, {}, {}
        for n, pc in enumerate(pieces):
            slot = int((n + 1) * len(stream) / len(pieces) - 3.5)
            placed.setdefault(max(2, min(slot, pv_slot[pc[:2]])), []).append(pc)

        def anchored(x, slot):
            deps = []
            for (u, j, pc) in placed.pop(slot, []):
                deps = vpu_piece(partial, u, j, pc, nought((u + 1) * n_kt + j))
            for mask, dep in zip(keeps, deps + after.pop(slot, [])):
                x = jnp.where(mask, x, dep if x.dtype == f32 else pltpu.bitcast(dep, u32))
            return x

        def prepare(u, j, dep):
            nh = u // n_qb + 1
            hn = head(nh * n_qb)
            g, lo = hn // hpg, (hn % hpg) * Dh
            step = (u % n_qb) * n_kt + j - 1
            rs = _share([b // 16 for (uu, _, b) in blocks if uu == 0], step, 58)
            if rs:
                idx = jnp.where(keeps[0], (lane + lo) & (LANES - 1), pltpu.bitcast(dep, i32))
                for r in rs:
                    khs[nh % 2][pl.ds(r * 8, 8), :] = _lane_gather(k_s[g, pl.ds(r * 8, 8), :], idx)
            cells = [(e, n, r) for e in range(8) for n in range(7) for r in range(voff[n_kt] // 16)]
            cells = _share(cells, step, 58)
            for e in sorted({c[0] for c in cells}):
                idx = jnp.where(keeps[0], jnp.full((8, LANES), lo + e, i32), pltpu.bitcast(dep, i32))
                for (_, n, r) in [c for c in cells if c[0] == e]:
                    kbs[nh % 2][0, n * 8 + e, pl.ds(r * 8, 8), :] = _lane_gather(kc_s[g, n, pl.ds(r * 8, 8), :], idx)
            for m in _share(list(range(14)), j - 1, 14):
                n, cols = m // 2, pl.ds((m % 2) * LANES, LANES)
                w = jnp.where(keeps[0], qc_s[(u + 1) % n_qb, head(u + 1), n, :, cols], dep)
                for e in range(8):
                    qbs[(u + 1) % 2][0, n * 8 + e, :, cols] = jnp.broadcast_to(w[e:e + 1], (8, LANES))

        probs = {blk: pend_s[pl.ds(n * 16, 16), :] for n, blk in enumerate(pending_in)}
        slot = done = 0
        while slot < len(stream):
            kind, what = stream[slot]
            if kind == "k":
                u, end = what[0], slot
                while stream[end][0] == "k" and stream[end][1][0] == u:
                    end += 1
                keys = [anchored(khs[(u // n_qb) % 2][pl.ds(stream[m][1][2] // 2, 8), :], m)
                        for m in range(slot, end)]
                s = _dot(_unpack(jnp.concatenate(keys, axis=0))[:, :Dh], q_rows(head(u), u % n_qb + nought(slot)))
                p = jnp.exp2(s)
                for n, m in enumerate(range(slot, end)):
                    probs[stream[m][1]] = p[n * 16:(n + 1) * 16]
                if slot == 0 or stream[slot - 1][0] == "v":
                    prepare(*divmod(done, n_kt), s[0:8, 0:LANES])
                slot = end
            else:
                u, j = what
                vt = v_rows(head(u), j * KC, KC)
                vt = jnp.concatenate([anchored(vt[0:8], slot), vt[8:16]], axis=0)
                l, acc = pv_tile(probs, partial, u, j, vt, l, acc)
                after[slot + 10] = [acc[0:8, BQ - LANES:BQ]]
                if j == n_kt - 1:
                    finish(head(u), u % n_qb, l, acc)
                slot += 1
                done += 1
        for n, blk in enumerate(pending_out):
            pend_s[pl.ds(n * 16, 16), :] = probs.pop(blk)
        assert not placed and not probs and not partial
        return l, acc

    @pl.when(jnp.logical_not(bounded))
    def _():
        lax.fori_loop(0, H * n_qb, max_subtracting_item, None)

    @pl.when(bounded)
    def _():
        l, acc = lax.fori_loop(0, H // HEADS_PER_STEP, bounded_heads,
                               (jnp.zeros((8, BQ), f32), jnp.zeros((Dh, BQ), f32)))
        u, j = tiles[-1]
        probs = {blk: pend_s[pl.ds(n * 16, 16), :] for n, blk in enumerate(pending_out) if blk[0] == u}
        partial = {}
        for pc in vpu_pieces(j):
            vpu_piece(partial, u, j, pc, 0)
        l, acc = pv_tile(probs, partial, u, j, v_rows(H - 1, j * KC, KC), l, acc)
        finish(H - 1, n_qb - 1, l, acc)

    b1 = b1_v[pl.ds(0, F)].astype(f32).reshape(1, F)
    b2 = b2_v[pl.ds(0, D)].astype(f32).reshape(1, D)
    out_cp = [pltpu.make_async_copy(out_v.at[pl.ds(n * rh, rh)], out_hbm.at[pl.ds(n * rh, rh)], out_sem.at[n])
              for n in range(2 * n_rc)]

    def o_jobs(r):
        def job(h0, q, dep=None):
            cols = pl.ds(q * LANES, LANES)
            ls = [l_s[r, h, :, cols] for h in range(h0, h0 + 8)]
            inv = 1.0 / _row_sums8([held(ls[0], dep)] + ls[1:])
            ot = [ot_s[r, pl.ds((h0 + n) * Dh, Dh), cols] * inv[n:n + 1] for n in range(8)]
            o = jnp.concatenate(ot, axis=0).astype(bf16).T
            xn_s[r][0, pl.ds(q * LANES // 2, LANES // 2), pl.ds(h0 * Dh, LANES)] = pltpu.bitcast(o, u32)

        return [functools.partial(job, h0, q) for q in range(n_qt) for h0 in range(0, H, 8)]

    def h_jobs(r):
        def job(t, dep):
            top, bot = (_layernorm(held(h_s[r + zero, pl.ds(r0, 16), :], dep)) for r0 in (t, rh + t))
            for n, a in enumerate(_strassen_lhs(top[:, :dh], top[:, dh:], bot[:, :dh], bot[:, dh:])):
                ha_s[r][0, n, pl.ds(t // 2, 8), :] = _pack(a)

        return [functools.partial(job, t) for t in range(0, rh, 16)]

    def out_proj(r, todo):
        for g in range(n_g):
            cols = pl.ds(g * LANES, LANES)
            y = _dot(_unpack(xn_s[r][g * zero]), wo_v[:, cols])
            _release(_share(todo, g, n_g - 1), y)
            h_s[r, :, cols] = x_v[pl.ds(r * RC, RC), cols].astype(f32) + y

    def ffn(r, todo):
        for c in range(0, fh, LANES):
            cols = pl.ds(c, LANES)
            u = _strassen(lambda n: _dot(_unpack(ha_s[r][(c // LANES + 1) * zero, n]), _unpack(w1_t[n, :, cols])),
                          (2, 4, 5, 1, 0, 3, 6))
            g = [_gelu2(u[q] + b1[:, (q % 2) * fh + c:(q % 2) * fh + c + LANES]) for q in range(4)]
            for n, a in enumerate(_strassen_lhs(*g)):
                ga_s[n, :, cols] = _pack(a)
        order = (2, 5, 0, 4, 1, 6, 3) if r + 1 < n_rc else (2, 5, 0, 1, 3, 4, 6)

        def product(n):
            m = _dot(_unpack(ga_s[n]), _unpack(w2_t[n]))
            _release(_share(todo, order.index(n), 6), m)
            return m

        y = _strassen(product, order)
        for q in (2, 3, 0, 1):
            r0, cols = (q // 2) * rh, pl.ds((q % 2) * dh, dh)
            res = 0.5 * y[q] + b2[:, (q % 2) * dh:(q % 2 + 1) * dh] + h_s[r + zero, pl.ds(r0, rh), cols]
            out_v[pl.ds(r * RC + r0, rh), cols] = res.astype(out_v.dtype)
            if q % 2:
                out_cp[2 * r + q // 2].start()

    _now(o_jobs(0))
    out_proj(0, o_jobs(1))
    for r in range(n_rc):
        if r + 1 < n_rc:
            out_proj(r + 1, h_jobs(0) if r == 0 else [])
        ffn(r, (o_jobs(r + 2) if r + 2 < n_rc else []) + (h_jobs(r + 1) if r + 1 < n_rc else []))
    for c in out_cp:
        c.wait()


@jax.jit
def pallas_sequential_preLN__softmax_full_mha__dense_activation_gelu__prompt_kernel(
    A_x: jax.Array,
    A_wqkv: jax.Array,
    A_wo: jax.Array,
    B_x: jax.Array,
    B_w1: jax.Array,
    B_b1: jax.Array,
    B_w2: jax.Array,
    B_b2: jax.Array,
):
    del B_x
    B, S, D = A_x.shape
    F = B_w1.shape[1]
    n_rc = S // RC
    assert (B, n_rc, S // KC, D // H, RC) == (1, 4, len(VPU_KEYS), 16, BQ)
    pairs = sum(VPU_KEYS) // 16
    V = pltpu.VMEM
    scratch = [
        V((S, D), A_x.dtype), V((3, D, D), A_wqkv.dtype), V((D, D), A_wo.dtype),
        V((D, F), B_w1.dtype), V((F, D), B_w2.dtype),
        V((D // 2, D), u32), V((D // 2, D), u32),
        V((7, D // 4, F // 2), u32), V((7, F // 4, D // 2), u32),
        *[V((1, RC // 2, D), u32) for _ in range(n_rc)],
        V((D // LANES, S // 2, LANES), u32),
        V((D // LANES, 7, -(-pairs // 4) * 32, LANES), f32),
        V((S // BQ, D // 2, BQ), u32),
        V((S // BQ, H, 8, 8, BQ // 2), f32),
        V((D, S), f32),
        V((S // BQ, D, BQ), f32),
        V((S // BQ, H, 8, BQ), f32),
        V((S // 2, LANES), u32), V((S // 2, LANES), u32),
        V((1, 56, pairs * 8, LANES), f32), V((1, 56, pairs * 8, LANES), f32),
        V((1, 56, 8, BQ // 2), f32), V((1, 56, 8, BQ // 2), f32),
        V((LAG_BLOCKS * 16, BQ), f32),
        V((S, BQ), f32),
        *[V((1, 7, RC // 4, D // 2), u32) for _ in range(n_rc)],
        V((n_rc, RC, D), f32),
        V((7, RC // 4, F // 2), u32),
        V((S, D), A_x.dtype),
        V((2048,), B_b1.dtype), V((2048,), B_b2.dtype),
        pltpu.SMEM((4,), i32),
        pltpu.SemaphoreType.DMA((8 + n_rc,)),
        pltpu.SemaphoreType.DMA((2 * n_rc,)),
    ]
    hbm = pl.BlockSpec(memory_space=pl.ANY)
    out = pl.pallas_call(
        _block_kernel,
        out_shape=jax.ShapeDtypeStruct((S, D), A_x.dtype),
        in_specs=[hbm] * 7,
        out_specs=hbm,
        scratch_shapes=scratch,
        compiler_params=pltpu.CompilerParams(vmem_limit_bytes=100 * 1024 * 1024),
        name="fused_block",
    )(A_x.reshape(S, D), A_wqkv, A_wo, B_w1, B_b1, B_w2, B_b2)
    return out.reshape(B, S, D)
```

```python
import functools
import math

import jax
import jax.numpy as jnp
from jax import lax
import jax.experimental.pallas as pl
import jax.experimental.pallas.tpu as pltpu

H = 32
EPS = 1e-5
LANES = 128
RC = 512
BQ = 512
KC = 128
VPU_KEYS = (16, 32, 16, 16, 32, 16, 16, 32, 16, 16, 32, 16, 16, 32, 16, 16)
HEADS_PER_STEP = 2
LAG_BLOCKS = 8
SAFE_LOG2 = 80.0

f32 = jnp.float32
bf16 = jnp.bfloat16
u32 = jnp.uint32
i32 = jnp.int32


def _layernorm(x):
    m = jnp.mean(x, axis=-1, keepdims=True)
    xc = x - m
    v = jnp.mean(xc * xc, axis=-1, keepdims=True)
    return xc * lax.rsqrt(v + EPS)


def _gelu2(u):
    c0 = math.sqrt(2.0 / math.pi)
    c1 = c0 * 0.044715
    return u + u * jnp.tanh(u * (c0 + c1 * (u * u)))


def _rows8(x):
    return [x[i:i + 8] for i in range(0, x.shape[0], 8)]


def _pack(x):
    return pltpu.bitcast(x.astype(bf16), u32)


def _unpack(w):
    return pltpu.bitcast(w, bf16)


def _dot(a, b):
    return jnp.dot(a, b, preferred_element_type=f32)


def _dot_nt(a, b):
    return lax.dot_general(a, b, (((1,), (1,)), ((), ())), preferred_element_type=f32)


def _lane_gather(x, idx):
    return jnp.take_along_axis(x, idx, axis=1, mode="promise_in_bounds", wrap_negative_indices=False)


def _strassen_lhs(a11, a12, a21, a22):
    return a11 + a22, a21 + a22, a11, a22, a11 + a12, a21 - a11, a12 - a22


def _strassen_rhs(b11, b12, b21, b22):
    return b11 + b22, b11, b12 - b22, b21 - b11, b22, b11 + b12, b21 + b22


_STRASSEN_USES = (((0, 1), (3, 1)), ((2, 1), (3, -1)), ((1, 1), (3, 1)), ((0, 1), (2, 1)),
                  ((0, -1), (1, 1)), ((3, 1),), ((0, 1),))


def _strassen(product, order):
    c = [None] * 4
    for n in order:
        m = product(n)
        for q, sign in _STRASSEN_USES[n]:
            if c[q] is None:
                c[q] = (m, sign)
            elif c[q][1] == sign:
                c[q] = (c[q][0] + m, sign)
            else:
                c[q] = (m - c[q][0] if sign > 0 else c[q][0] - m, 1)
    assert all(sign > 0 for _, sign in c)
    return [v for v, _ in c]


def _row_sums8(xs):
    row = lax.broadcasted_iota(i32, xs[0].shape, 0)
    c = [jnp.where(row < 4, a, b) + pltpu.roll(jnp.where(row < 4, b, a), 4, 0)
         for a, b in zip(xs[:4], xs[4:])]
    for sh in (2, 1):
        low = (row & sh) == 0
        n = len(c) // 2
        c = [jnp.where(low, a, b) + jnp.where(low, pltpu.roll(a, 8 - sh, 0), pltpu.roll(b, sh, 0))
             for a, b in zip(c[:n], c[n:])]
    return c[0]


def _share(todo, n, parts):
    return todo[n * len(todo) // parts:(n + 1) * len(todo) // parts] if 0 <= n < parts else []


def _now(todo):
    for job in todo:
        job()


def _release(todo, y):
    vregs = [(t, c) for c in range(0, y.shape[1], LANES) for t in range(0, y.shape[0], 8)]
    for n, job in enumerate(todo):
        t, c = vregs[n * len(vregs) // len(todo)]
        job(y[t:t + 8, c:c + LANES])


def _block_kernel(x_hbm, wqkv_hbm, wo_hbm, w1_hbm, b1_hbm, w2_hbm, b2_hbm, out_hbm,
                  x_v, wqkv_v, wo_v, w1_v, w2_v, wqt_s, wvt_s, w1_t, w2_t,
                  xn_0, xn_1, xn_2, xn_3, k_s, kc_s, qt_s, qc_s, vt_s, ot_s, l_s,
                  kh_a, kh_b, kb_a, kb_b, qb_a, qb_b, pend_s, s_s,
                  ha_0, ha_1, ha_2, ha_3, h_s, ga_s, out_v, b1_v, b2_v, zero_s, in_sem, out_sem):
    S, D = x_v.shape
    F = w1_v.shape[1]
    Dh = D // H
    n_rc, n_qb, n_kt, n_qt, n_g = S // RC, S // BQ, S // KC, BQ // LANES, D // LANES
    hpg = LANES // Dh
    rh, dh, fh = RC // 2, D // 2, F // 2
    vk = VPU_KEYS
    voff = [sum(vk[:j]) for j in range(n_kt + 1)]
    xn_s = [xn_0, xn_1, xn_2, xn_3]
    ha_s = [ha_0, ha_1, ha_2, ha_3]

    def copy(src, dst, n):
        return pltpu.make_async_copy(src, dst, in_sem.at[n])

    wq_cp, wk_cp, wv_cp = (copy(wqkv_hbm.at[:, pl.ds(n * D, D)], wqkv_v.at[n], n) for n in range(3))
    ffn_cp = [copy(wo_hbm, wo_v, 3), copy(w1_hbm, w1_v, 4), copy(w2_hbm, w2_v, 5),
              copy(b1_hbm, b1_v.at[pl.ds(0, F)], 6), copy(b2_hbm, b2_v.at[pl.ds(0, D)], 7)]
    x_cp = [copy(x_hbm.at[pl.ds(r * RC, RC)], x_v.at[pl.ds(r * RC, RC)], 8 + r) for r in range(n_rc)]
    for c in x_cp[:1] + [wk_cp] + x_cp[1:] + [wq_cp, wv_cp] + ffn_cp:
        c.start()

    def put_zero(n, _):
        zero_s[n] = n // 65536

    lax.fori_loop(0, zero_s.shape[0], put_zero, None)
    zero = zero_s[0]
    keep = lax.broadcasted_iota(i32, (8, LANES), 0) >= zero

    def held(x, dep):
        if dep is None:
            return x
        head = jnp.concatenate([jnp.where(keep, t, dep) for t in _rows8(x[:, :LANES])], axis=0)
        return jnp.concatenate([head, x[:, LANES:]], axis=1) if x.shape[1] > LANES else head

    def weight_jobs(ref, table):
        kh, nh = ref.shape[0] // 2, ref.shape[1] // 2

        def job(t, c, dep):
            words = [pltpu.bitcast(ref[pl.ds(a * kh + t, 16), pl.ds(b * nh + c, LANES)], u32)
                     for a in range(2) for b in range(2)]
            words = [jnp.where(keep, w, pltpu.bitcast(dep, u32)) for w in words]
            blocks = [_unpack(w).astype(f32) for w in words]
            for n, b in enumerate(_strassen_rhs(*blocks)):
                same = [w for w, blk in zip(words, blocks) if blk is b]
                table[n, pl.ds(t // 2, 8), pl.ds(c, LANES)] = same[0] if same else _pack(b)

        return [functools.partial(job, t, c) for t in range(0, kh, 16) for c in range(0, nh, LANES)]

    peaks = {}

    def peak(name, w):
        peaks[name] = w if name not in peaks else jnp.maximum(peaks[name], w)

    def x_jobs(r, rows=32):
        def job(t, dep=None):
            xn = _layernorm(held(x_v[pl.ds(r * RC + t, rows), :].astype(f32), dep))
            xn_s[r][0, pl.ds(t // 2, rows // 2), :] = _pack(xn)

        return [functools.partial(job, t) for t in range(0, RC, rows)]

    k_squares, k_pairs = [], []

    def project_k(r, g, todo=()):
        k = _dot(_unpack(xn_s[r][g * zero]), wqkv_v[1, :, pl.ds(g * LANES, LANES)])
        _release(todo, k)
        k_s[g, pl.ds(r * RC // 2, RC // 2), :] = _pack(k)
        for t0 in range(0, RC, KC):
            j = (r * RC + t0) // KC
            for t in range(0, vk[j], 16):
                k_pairs.append((g, (voff[j] + t) // 2, k[t0 + t:t0 + t + 8], k[t0 + t + 8:t0 + t + 16]))
        k2 = _rows8(k * k)
        k_squares.extend(functools.reduce(jnp.maximum, k2[n:n + 8]) for n in range(0, len(k2), 8))

    def key_operands(g, row, a11, a21, dep):
        a11, a21 = held(a11, dep), held(a21, dep)
        a12, a22 = (pltpu.roll(a, LANES - Dh // 2, 1) for a in (a11, a21))
        s1 = a21 + a22
        s2 = s1 - a11
        for n, t in enumerate((a11, a12, a12 - s2, a22, s1, s2, a11 - a21)):
            kc_s[g, n, pl.ds(row, 8), :] = t

    def key_peak(w, dep):
        w = held(w, dep)
        for sh in (1, 2, 4, 8):
            w = w + pltpu.roll(w, sh, 1)
        peak("k", w)

    def first_tables(n, e, dep):
        kc = held(kc_s[0, n, pl.ds(0, voff[n_kt] // 2), :], dep)
        kb_a[0, n * 8 + e] = jnp.broadcast_to(kc[:, e:e + 1], kc.shape)
        qb_a[0, n * 8 + e] = jnp.broadcast_to(qc_s[0, 0, n, e:e + 1, :], (8, BQ // 2))

    def project_q(r, todo):
        qt = _dot_nt(_unpack(wqt_s[...]), _unpack(xn_s[r][0]))
        _release(todo, qt)
        qt = qt * ((Dh ** -0.5) * math.log2(math.e))
        qt_s[r] = _pack(qt)
        squares = []
        for h in range(H):
            lo, hi = _rows8(qt[h * Dh:(h + 1) * Dh])
            b11, b12, b21, b22 = (jnp.concatenate([t[:, c * LANES:(c + 1) * LANES] for c in (c0, c0 + 2)], axis=1)
                                  for t in (lo, hi) for c0 in range(2))
            t1 = b12 - b11
            t2 = b22 - t1
            for n, t in enumerate((b11, b21, b22, b21 - t2, t1, t2, b22 - b12)):
                qc_s[r, h, n] = t
            squares.append(lo * lo + hi * hi)
        for h0 in range(0, H, 8):
            peak("q", _row_sums8(squares[h0:h0 + 8]))

    def project_v(r, todo):
        vt = _dot_nt(_unpack(wvt_s[...]), _unpack(xn_s[r][0]))
        _release(todo, vt)
        vt_s[:, pl.ds(r * RC, RC)] = vt
        peak("v", functools.reduce(jnp.maximum, _rows8(jnp.abs(vt))))

    n_it = HEADS_PER_STEP * n_qb
    khs, kbs, qbs = [kh_a, kh_b], [kb_a, kb_b], [qb_a, qb_b]
    blocks = [(u, j, j * KC + b) for u in range(-1, n_it + 1) for j in range(n_kt)
              for b in range(KC - 16, vk[j] - 1, -16)]
    tile_end = {(u, j): n + 1 for n, (u, j, _) in enumerate(blocks)}
    tiles = [(-1, n_kt - 1)] + [(u, j) for u in range(n_it) for j in range(n_kt)]
    stream, n_streamed = [], tile_end[-1, n_kt - 2] + LAG_BLOCKS
    pending_in = blocks[tile_end[-1, n_kt - 2]:n_streamed]
    pending_in += [(-1, n_kt - 1, S - KC + t) for t in range(0, vk[-1], 16)]
    for tile in tiles[:-1]:
        stream += [("k", blk) for blk in blocks[n_streamed:tile_end[tile] + LAG_BLOCKS]] + [("v", tile)]
        n_streamed = tile_end[tile] + LAG_BLOCKS
    pending_out = blocks[tile_end[n_it - 1, n_kt - 2]:n_streamed]
    pending_out += [(n_it - 1, n_kt - 1, S - KC + t) for t in range(0, vk[-1], 16)]

    def q_rows(h, qb):
        return _unpack(qt_s[qb, pl.ds(pl.multiple_of(h * (Dh // 2), Dh // 2), Dh // 2), :])

    def start_stream():
        for n, (u, _, b) in enumerate(pending_in):
            if u < 0:
                pend_s[pl.ds(n * 16, 16), :] = jnp.zeros((16, BQ), f32)
            else:
                s = _dot(_unpack(k_s[0, pl.ds(b // 2, 8), :])[:, :Dh], q_rows(0, 0))
                pend_s[pl.ds(n * 16, 16), :] = jnp.exp2(s)

    x_cp[0].wait()
    _now(x_jobs(0, RC))
    wk_cp.wait()
    project_k(0, 0)
    project_k(0, 1)
    x_cp[1].wait()
    todo = x_jobs(1)
    _now(todo[:3])
    project_k(0, 2, todo[3:10])
    project_k(0, 3, todo[10:])
    project_k(1, 0)
    project_k(1, 1)
    x_cp[2].wait()
    todo = x_jobs(2)
    _now(todo[:3])
    project_k(1, 2, todo[3:10])
    project_k(1, 3, todo[10:])
    project_k(2, 0)
    project_k(2, 1)
    x_cp[3].wait()
    wq_cp.wait()
    todo = x_jobs(3)
    _now(todo[:3])
    project_k(2, 2, todo[3:10])
    project_k(2, 3, todo[10:])
    wqt_s[...] = pltpu.bitcast(wqkv_v[0].T, u32)
    for g in range(n_g):
        project_k(3, g)
    project_q(0, [functools.partial(key_operands, *args) for args in sorted(k_pairs, key=lambda a: a[:2])])
    project_q(1, [functools.partial(key_peak, w) for w in k_squares])
    kh_a[...] = k_s[0]
    todo = [functools.partial(first_tables, n, e) for e in range(8) for n in range(7)]
    project_q(2, _share(todo, 0, 2))
    for c in [wv_cp] + ffn_cp:
        c.wait()
    wvt_s[...] = pltpu.bitcast(wqkv_v[2].T, u32)
    project_q(3, _share(todo, 1, 2))
    start_stream()
    todo = weight_jobs(w1_v, w1_t) + weight_jobs(w2_v, w2_t)
    for r in range(n_rc):
        project_v(r, _share(todo, r, n_rc))

    v_peak = jnp.max(peaks["v"])
    bounded = ((jnp.max(peaks["k"]) * jnp.max(peaks["q"]) <= SAFE_LOG2 * SAFE_LOG2)
               & (v_peak <= 2.0 ** 30) & (v_peak >= 2.0 ** -20))

    def v_rows(h, start, size):
        return vt_s[pl.ds(pl.multiple_of(h * Dh, Dh), Dh), pl.ds(start, size)]

    def finish(h, qb, l, acc):
        ot_s[qb, pl.ds(pl.multiple_of(h * Dh, Dh), Dh), :] = acc
        l_s[qb, h] = l

    def max_subtracting_item(it, _):
        h, qb = it // n_qb, it % n_qb

        @pl.when(qb == 0)
        def _():
            kh_a[...] = pltpu.roll(k_s[h // hpg], (LANES - (h % hpg) * Dh) % LANES, 1)

        qh = q_rows(h, qb)
        step = 4 * KC

        def scores(c, m):
            keys = kh_a[pl.ds(pl.multiple_of(c * (step // 2), step // 2), step // 2), :]
            s = _dot(_unpack(keys)[:, :Dh], qh)
            s_s[pl.ds(pl.multiple_of(c * step, step), step), :] = s
            return functools.reduce(jnp.maximum, [m] + _rows8(s))

        m = lax.fori_loop(0, S // step, scores, jnp.full((8, BQ), -jnp.inf, f32))
        m = jnp.max(m, axis=0, keepdims=True)

        def values(c, carry):
            l, acc = carry
            r0 = pl.multiple_of(c * step, step)
            p = jnp.exp2(s_s[pl.ds(r0, step), :] - m)
            return functools.reduce(jnp.add, [l] + _rows8(p)), acc + _dot(v_rows(h, r0, step), p)

        l, acc = lax.fori_loop(0, S // step, values, (jnp.zeros((8, BQ), f32), jnp.zeros((Dh, BQ), f32)))
        finish(h, qb, l, acc)

    def vpu_pieces(j):
        return [(t, n) for t in range(0, vk[j], 16) for n in range(7)]

    def vpu_piece(partial, u, j, piece, z):
        t, n = piece
        kb, qb = kbs[(u // n_qb) % 2], qbs[u % 2]
        a = partial.setdefault((u, j, t), {})
        marks = []

        def product(m, acc=None):
            for e in range(8):
                kk = kb[z, m * 8 + e, pl.ds((voff[j] + t) // 2, 8), :]
                term = jnp.concatenate([kk, kk], axis=1) * qb[z, m * 8 + e]
                acc = term if acc is None else acc + term
                if e == 6:
                    marks.extend([acc[:, :LANES], acc[:, LANES:]])
            return acc

        if n == 0:
            a["p1"] = product(0)
        elif n == 1:
            a["c11"] = product(1, a["p1"])
        elif n == 2:
            a["u2"] = product(5, a["p1"])
        elif n == 3:
            a["p5"] = product(4)
        elif n == 4:
            a["u3"] = product(6, a["u2"])
            a["u4"] = a["u2"] + a["p5"]
            a["c22"] = a["u3"] + a["p5"]
        elif n == 5:
            a["c12"] = product(2, a["u4"])
        else:
            a["c21"] = product(3, a["u3"])
        return marks

    def vpu_probs(probs, partial, u, j):
        for t in range(0, vk[j], 16):
            a = partial.pop((u, j, t))
            rows = [jnp.exp2(jnp.concatenate([a[name][:, c:c + LANES] for c in (0, LANES) for name in names], axis=1))
                    for names in (("c11", "c12"), ("c21", "c22"))]
            probs[u, j, j * KC + t] = jnp.concatenate(rows, axis=0)

    def pv_tile(probs, u, j, vt, l, acc):
        p = jnp.concatenate([probs.pop((u, j, j * KC + b)) for b in range(0, KC, 16)], axis=0)
        l = functools.reduce(jnp.add, ([] if j == 0 else [l]) + _rows8(p)[::-1])
        pv = _dot(vt, p)
        return l, (pv if j == 0 else acc + pv)

    def bounded_heads(i, carry):
        l, acc = carry
        row = lax.broadcasted_iota(i32, (8, LANES), 0)
        lane = lax.broadcasted_iota(i32, (8, LANES), 1)
        always = row > (i // 65536 - 1)

        def nought(t):
            return (i * 4096 + t) // (4096 * H)

        def head(u):
            return jnp.clip(HEADS_PER_STEP * i + u // n_qb, 0, H - 1)

        pieces = [(u, j, pc) for (u, j) in tiles[1:] for pc in vpu_pieces(j)]
        pv_slot = {what: n for n, (kind, what) in enumerate(stream) if kind == "v"}
        spots = [(m + r / 2, m, r) for m, (kind, _) in enumerate(stream) if kind == "k" for r in range(2)]
        placed, after, partial = {}, {}, {}
        for n, pc in enumerate(pieces):
            when = (n + 1 + len(vpu_pieces(n_kt - 1))) * len(stream) / len(pieces) - 12.5
            when = min(when, pv_slot.get(pc[:2], math.inf) - 10)
            _, m, r = min(spots, key=lambda spot: abs(spot[0] - when))
            placed.setdefault((m, r), []).append(pc)

        def anchored(p, m):
            rows = []
            for r, p8 in enumerate(_rows8(p)):
                deps = [dep for (u, j, pc) in placed.pop((m, r), [])
                        for dep in vpu_piece(partial, u, j, pc, nought((u + 1) * n_kt + j))]
                if r == 1 and m in after:
                    deps.append(after.pop(m))
                if deps:
                    cells = [p8[:, c:c + LANES] for c in range(0, BQ, LANES)]
                    for k, dep in enumerate(deps[-n_qt:]):
                        c = (k + 2 * (2 * m + r)) % n_qt
                        cells[c] = jnp.where(always, cells[c], dep)
                    p8 = jnp.concatenate(cells, axis=1)
                rows.append(p8)
            return jnp.concatenate(rows, axis=0)

        def prepare(u, j, dep):
            nh = u // n_qb + 1
            hn = head(nh * n_qb)
            g, lo = hn // hpg, (hn % hpg) * Dh
            step = (u % n_qb) * n_kt + j - 1
            rs = _share([b // 16 for (uu, _, b) in blocks if uu == 0], step, 56)
            if rs:
                idx = jnp.where(always, (lane + lo) & (LANES - 1), pltpu.bitcast(dep, i32))
                for r in rs:
                    khs[nh % 2][pl.ds(r * 8, 8), :] = _lane_gather(k_s[g, pl.ds(r * 8, 8), :], idx)
            cells = [(e, n, r) for e in range(8) for n in range(7) for r in range(voff[n_kt] // 16)]
            cells = _share(cells, step, 56)
            for e in sorted({c[0] for c in cells}):
                idx = jnp.where(always, jnp.full((8, LANES), lo + e, i32), pltpu.bitcast(dep, i32))
                for (_, n, r) in [c for c in cells if c[0] == e]:
                    kbs[nh % 2][0, n * 8 + e, pl.ds(r * 8, 8), :] = _lane_gather(kc_s[g, n, pl.ds(r * 8, 8), :], idx)
            for m in _share(list(range(14)), j - 1, 12):
                n, cols = m // 2, pl.ds((m % 2) * LANES, LANES)
                w = jnp.where(always, qc_s[(u + 1) % n_qb, head(u + 1), n, :, cols], dep)
                for e in range(8):
                    qbs[(u + 1) % 2][0, n * 8 + e, :, cols] = jnp.broadcast_to(w[e:e + 1], (8, LANES))

        probs = {blk: pend_s[pl.ds(n * 16, 16), :] for n, blk in enumerate(pending_in)}
        slot = done = 0
        while slot < len(stream):
            kind, what = stream[slot]
            if kind == "k":
                u, end = what[0], slot
                while stream[end][0] == "k" and stream[end][1][0] == u:
                    end += 1
                keys = [khs[(u // n_qb) % 2][pl.ds(stream[m][1][2] // 2, 8), :] for m in range(slot, end)]
                s = _dot(_unpack(jnp.concatenate(keys, axis=0))[:, :Dh], q_rows(head(u), u % n_qb + nought(slot)))
                p = jnp.exp2(s)
                for n, m in enumerate(range(slot, end)):
                    probs[stream[m][1]] = anchored(p[n * 16:(n + 1) * 16], m)
                if slot == 0 or stream[slot - 1][0] == "v":
                    latest = s[0:8, 0:LANES]
                    prepare(*divmod(done, n_kt), latest)
                slot = end
            else:
                u, j = what
                vt = v_rows(head(u), j * KC, KC)
                if u >= 0:
                    vpu_probs(probs, partial, u, j)
                l, acc = pv_tile(probs, u, j, vt, l, acc)
                after[slot + 1] = acc[0:8, BQ - LANES:BQ]
                if j == n_kt - 1:
                    finish(head(u), u % n_qb, l, acc)
                slot += 1
                done += 1
        for key, a in partial.items():
            partial[key] = {name: jnp.concatenate([jnp.where(always, a[name][:, c:c + LANES], latest)
                                                   for c in (0, LANES)], axis=1)
                            for name in ("c11", "c12", "c21", "c22")}
        vpu_probs(probs, partial, *tiles[-1])
        for n, blk in enumerate(pending_out):
            pend_s[pl.ds(n * 16, 16), :] = probs.pop(blk)
        assert not placed and not probs and not partial
        return l, acc

    @pl.when(jnp.logical_not(bounded))
    def _():
        lax.fori_loop(0, H * n_qb, max_subtracting_item, None)

    @pl.when(bounded)
    def _():
        l, acc = lax.fori_loop(0, H // HEADS_PER_STEP, bounded_heads,
                               (jnp.zeros((8, BQ), f32), jnp.zeros((Dh, BQ), f32)))
        u, j = tiles[-1]
        probs = {blk: pend_s[pl.ds(n * 16, 16), :] for n, blk in enumerate(pending_out) if blk[0] == u}
        l, acc = pv_tile(probs, u, j, v_rows(H - 1, j * KC, KC), l, acc)
        finish(H - 1, n_qb - 1, l, acc)

    b1 = b1_v[pl.ds(0, F)].astype(f32).reshape(1, F)
    b2 = b2_v[pl.ds(0, D)].astype(f32).reshape(1, D)
    out_cp = [pltpu.make_async_copy(out_v.at[pl.ds(n * rh, rh)], out_hbm.at[pl.ds(n * rh, rh)], out_sem.at[n])
              for n in range(2 * n_rc)]

    def o_jobs(r):
        def job(h0, q, dep=None):
            cols = pl.ds(q * LANES, LANES)
            ls = [l_s[r, h, :, cols] for h in range(h0, h0 + 8)]
            inv = 1.0 / _row_sums8([held(ls[0], dep)] + ls[1:])
            ot = [ot_s[r, pl.ds((h0 + n) * Dh, Dh), cols] * inv[n:n + 1] for n in range(8)]
            o = jnp.concatenate(ot, axis=0).astype(bf16).T
            xn_s[r][0, pl.ds(q * LANES // 2, LANES // 2), pl.ds(h0 * Dh, LANES)] = pltpu.bitcast(o, u32)

        return [functools.partial(job, h0, q) for q in range(n_qt) for h0 in range(0, H, 8)]

    def h_jobs(r):
        def job(t, dep):
            top, bot = (_layernorm(held(h_s[r + zero, pl.ds(r0, 16), :], dep)) for r0 in (t, rh + t))
            for n, a in enumerate(_strassen_lhs(top[:, :dh], top[:, dh:], bot[:, :dh], bot[:, dh:])):
                ha_s[r][0, n, pl.ds(t // 2, 8), :] = _pack(a)

        return [functools.partial(job, t) for t in range(0, rh, 16)]

    def out_proj(r, todo):
        for g in range(n_g):
            cols = pl.ds(g * LANES, LANES)
            y = _dot(_unpack(xn_s[r][g * zero]), wo_v[:, cols])
            _release(_share(todo, g, n_g - 1), y)
            h_s[r, :, cols] = x_v[pl.ds(r * RC, RC), cols].astype(f32) + y

    def ffn(r, todo):
        for c in range(0, fh, LANES):
            cols = pl.ds(c, LANES)
            u = _strassen(lambda n: _dot(_unpack(ha_s[r][(c // LANES + 1) * zero, n]), _unpack(w1_t[n, :, cols])),
                          (2, 4, 5, 1, 0, 3, 6))
            g = [_gelu2(u[q] + b1[:, (q % 2) * fh + c:(q % 2) * fh + c + LANES]) for q in range(4)]
            for n, a in enumerate(_strassen_lhs(*g)):
                ga_s[n, :, cols] = _pack(a)
        order = (2, 5, 0, 4, 1, 6, 3) if r + 1 < n_rc else (2, 5, 0, 1, 3, 4, 6)

        def product(n):
            m = _dot(_unpack(ga_s[n]), _unpack(w2_t[n]))
            _release(_share(todo, order.index(n), 6), m)
            return m

        y = _strassen(product, order)
        for q in (2, 3, 0, 1):
            r0, cols = (q // 2) * rh, pl.ds((q % 2) * dh, dh)
            res = 0.5 * y[q] + b2[:, (q % 2) * dh:(q % 2 + 1) * dh] + h_s[r + zero, pl.ds(r0, rh), cols]
            out_v[pl.ds(r * RC + r0, rh), cols] = res.astype(out_v.dtype)
            if q % 2:
                out_cp[2 * r + q // 2].start()

    _now(o_jobs(0))
    out_proj(0, o_jobs(1))
    for r in range(n_rc):
        if r + 1 < n_rc:
            out_proj(r + 1, h_jobs(0) if r == 0 else [])
        ffn(r, (o_jobs(r + 2) if r + 2 < n_rc else []) + (h_jobs(r + 1) if r + 1 < n_rc else []))
    for c in out_cp:
        c.wait()


@jax.jit
def pallas_sequential_preLN__softmax_full_mha__dense_activation_gelu__prompt_kernel(
    A_x: jax.Array,
    A_wqkv: jax.Array,
    A_wo: jax.Array,
    B_x: jax.Array,
    B_w1: jax.Array,
    B_b1: jax.Array,
    B_w2: jax.Array,
    B_b2: jax.Array,
):
    del B_x
    B, S, D = A_x.shape
    F = B_w1.shape[1]
    n_rc = S // RC
    assert (B, n_rc, S // KC, D // H, RC) == (1, 4, len(VPU_KEYS), 16, BQ)
    pairs = sum(VPU_KEYS) // 16
    V = pltpu.VMEM
    scratch = [
        V((S, D), A_x.dtype), V((3, D, D), A_wqkv.dtype), V((D, D), A_wo.dtype),
        V((D, F), B_w1.dtype), V((F, D), B_w2.dtype),
        V((D // 2, D), u32), V((D // 2, D), u32),
        V((7, D // 4, F // 2), u32), V((7, F // 4, D // 2), u32),
        *[V((1, RC // 2, D), u32) for _ in range(n_rc)],
        V((D // LANES, S // 2, LANES), u32),
        V((D // LANES, 7, -(-pairs // 4) * 32, LANES), f32),
        V((S // BQ, D // 2, BQ), u32),
        V((S // BQ, H, 8, 8, BQ // 2), f32),
        V((D, S), f32),
        V((S // BQ, D, BQ), f32),
        V((S // BQ, H, 8, BQ), f32),
        V((S // 2, LANES), u32), V((S // 2, LANES), u32),
        V((1, 56, pairs * 8, LANES), f32), V((1, 56, pairs * 8, LANES), f32),
        V((1, 56, 8, BQ // 2), f32), V((1, 56, 8, BQ // 2), f32),
        V((LAG_BLOCKS * 16 + VPU_KEYS[-1], BQ), f32),
        V((S, BQ), f32),
        *[V((1, 7, RC // 4, D // 2), u32) for _ in range(n_rc)],
        V((n_rc, RC, D), f32),
        V((7, RC // 4, F // 2), u32),
        V((S, D), A_x.dtype),
        V((2048,), B_b1.dtype), V((2048,), B_b2.dtype),
        pltpu.SMEM((4,), i32),
        pltpu.SemaphoreType.DMA((8 + n_rc,)),
        pltpu.SemaphoreType.DMA((2 * n_rc,)),
    ]
    hbm = pl.BlockSpec(memory_space=pl.ANY)
    out = pl.pallas_call(
        _block_kernel,
        out_shape=jax.ShapeDtypeStruct((S, D), A_x.dtype),
        in_specs=[hbm] * 7,
        out_specs=hbm,
        scratch_shapes=scratch,
        compiler_params=pltpu.CompilerParams(vmem_limit_bytes=100 * 1024 * 1024),
        name="fused_block",
    )(A_x.reshape(S, D), A_wqkv, A_wo, B_w1, B_b1, B_w2, B_b2)
    return out.reshape(B, S, D)
```
